```python
import jax
import jax.numpy as jnp

def _softmax(x, axis=-1):
    return jax.nn.softmax(x, axis=axis)
def _gelu(x):
    return jax.nn.gelu(x, approximate=True)
def _silu(x):
    return jax.nn.silu(x)
def _sigmoid(x):
    return jax.nn.sigmoid(x)
def _layernorm(x, axis=-1, eps=1e-5):
    m = jnp.mean(x, axis=axis, keepdims=True)
    v = jnp.var(x, axis=axis, keepdims=True)
    return (x - m) / jnp.sqrt(v + eps)
def _scatter_add(tgt, idx, src, axis=0):
    return tgt.at[idx].add(src)
def _segment_sum(src, seg, n):
    return jax.ops.segment_sum(src, seg, n)
class _Rng:
    def __init__(self, key):
        self._k = key
    def _next(self):
        self._k, sub = jax.random.split(self._k)
        return sub
    def normal(self, shape):
        return jax.random.normal(self._next(), shape, dtype=jnp.bfloat16)
    def randint(self, lo, hi, shape):
        return jax.random.randint(self._next(), shape, lo, hi, dtype=jnp.int32)
    def uniform(self, shape, lo=0.0, hi=1.0):
        return jax.random.uniform(self._next(), shape, jnp.bfloat16, lo, hi)
    def permutation(self, n):
        return jax.random.permutation(self._next(), n)


kernel_name = 'sequential_preLN__mha_block_cached__moe_arch_mod__decode'

def setup_inputs():
    _rng = _Rng(jax.random.key(int.from_bytes(__import__("os").urandom(4), "little")))
    _w = (lambda a: (lambda t: t.astype(jnp.bfloat16) if jnp.issubdtype(t.dtype, jnp.floating) else t)(jnp.asarray(a)))
    def _A_setup():
        B, Sq, D = 4, 1, 640
        H, Sk, Dh = 32, 8192, 192
        return {
            "x": _w((lambda *s: _rng.normal(s) * 0.05)(B, Sq, D)),
            "k_cache": _w((lambda *s: _rng.normal(s) * 0.05)(B, H, Sk, Dh)),
            "v_cache": _w((lambda *s: _rng.normal(s) * 0.05)(B, H, Sk, Dh)),
            "wq": _w((lambda *s: _rng.normal(s) * 0.05)(D, H * Dh) * (D ** -0.5)),
            "wo": _w((lambda *s: _rng.normal(s) * 0.05)(H * Dh, D) * ((H * Dh) ** -0.5)),
        }
    _A_in = _A_setup()

    def _B_setup():
        B, S, D, F, C = 4, 1, 640, 1536, 1
        return {
            "x": _w((lambda *s: _rng.normal(s) * 0.05)(B, S, D)),
            "w_r": _w((lambda *s: _rng.normal(s) * 0.05)(D)),
            "w_gate": _w((lambda *s: _rng.normal(s) * 0.05)(D, F)),
            "w_up": _w((lambda *s: _rng.normal(s) * 0.05)(D, F)),
            "w_down": _w((lambda *s: _rng.normal(s) * 0.05)(F, D)),
        }
    _B_in = _B_setup()

    return {
        "A_x": _A_in["x"],
        "A_k_cache": _A_in["k_cache"],
        "A_v_cache": _A_in["v_cache"],
        "A_wq": _A_in["wq"],
        "A_wo": _A_in["wo"],
        "B_x": _B_in["x"],
        "B_w_r": _B_in["w_r"],
        "B_w_gate": _B_in["w_gate"],
        "B_w_up": _B_in["w_up"],
        "B_w_down": _B_in["w_down"],
    }

def reference(A_x, A_k_cache, A_v_cache, A_wq, A_wo, B_x, B_w_r, B_w_gate, B_w_up, B_w_down):
    def _A_ref(x, k_cache, v_cache, wq, wo):
        B, Sq, D = x.shape
        H, Dh = 32, 192
        q = (lambda x, *d: x.transpose(*d))((x @ wq).reshape(B, Sq, H, Dh), 0, 2, 1, 3)
        scores = jnp.einsum("bhqd,bhkd->bhqk", q, k_cache) * (Dh ** -0.5)
        p = _softmax(scores, axis=-1)
        o = jnp.einsum("bhqk,bhkd->bhqd", p, v_cache)
        return (lambda x, *d: x.transpose(*d))(o, 0, 2, 1, 3).reshape(B, Sq, H * Dh) @ wo

    def _B_ref(x, w_r, w_gate, w_up, w_down):
        B, S, D = x.shape
        C = 1
        r = x @ w_r
        idx = jnp.argsort(-r, axis=-1)[:, :C]
        idx_e = jnp.repeat(idx.reshape(B, C, 1), D, axis=2)
        x_sel = jnp.take_along_axis(x, idx_e, axis=1)
        g = _silu(x_sel @ w_gate)
        u = x_sel @ w_up
        y = (g * u) @ w_down
        r_sel = _sigmoid(jnp.take_along_axis(r, idx, axis=1))
        y = y * r_sel.reshape(B, C, 1)
        b_off = (jnp.arange(B) * S).reshape(B, 1)
        flat_idx = (idx + b_off).reshape(B * C)
        zero = (x * 0.0).reshape(B * S, D)
        upd = _scatter_add(zero, flat_idx, y.reshape(B * C, D), axis=0)
        return x + upd.reshape(B, S, D)

    x = A_x
    h = x + _A_ref(_layernorm(x, axis=-1), A_k_cache, A_v_cache, A_wq, A_wo)
    h2 = h + _B_ref(_layernorm(h, axis=-1), B_w_r, B_w_gate, B_w_up, B_w_down)
    return h2
```

```python
import functools

import jax
import jax.numpy as jnp
from jax import lax
import jax.experimental.pallas as pl
import jax.experimental.pallas.tpu as pltpu

B, H, SK, DH, D, F = 4, 32, 8192, 192, 640, 1536
NSTEP = B * H
ROWS = 8
EPS = 1e-5
SCALE = DH ** -0.5
PAIR = 2 * DH


def _layernorm(x):
    m = jnp.mean(x, axis=-1, keepdims=True)
    c = x - m
    v = jnp.mean(c * c, axis=-1, keepdims=True)
    return c / jnp.sqrt(v + EPS)


def _make_kernel(vchunks):
    vrows = DH // vchunks

    def kernel(x_hbm, k_hbm, v_hbm, wq_hbm, wo_hbm, wr_hbm, wg_hbm, wu_hbm, wd_hbm,
               out_ref,
               x_v, wr_v, wq_v, wo_v, wg_v, wu_v, wd_v, kbuf, vbuf,
               x_s, xn_s, q_s, o_s, acc_s,
               sem_w, sem_k, sem_v):
        def k_copy(t, slot):
            return pltpu.make_async_copy(
                k_hbm.at[t % B, t // B], kbuf.at[slot], sem_k.at[slot])

        def v_copy(t, slot, c):
            return pltpu.make_async_copy(
                v_hbm.at[t % B, t // B, pl.ds(c * vrows, vrows)],
                vbuf.at[slot, pl.ds(c * vrows, vrows)], sem_v.at[slot, c])

        x_cp = pltpu.make_async_copy(x_hbm, x_v, sem_w.at[0])
        wq0_cp = pltpu.make_async_copy(
            wq_hbm.at[:, pl.ds(0, PAIR)], wq_v.at[:, pl.ds(0, PAIR)], sem_w.at[1])
        wq1_cp = pltpu.make_async_copy(
            wq_hbm.at[:, pl.ds(PAIR, H * DH - PAIR)],
            wq_v.at[:, pl.ds(PAIR, H * DH - PAIR)], sem_w.at[2])
        wo_cp = pltpu.make_async_copy(wo_hbm, wo_v, sem_w.at[3])
        wr_cp = pltpu.make_async_copy(wr_hbm, wr_v, sem_w.at[4])
        wg_cp = pltpu.make_async_copy(wg_hbm, wg_v, sem_w.at[5])
        wu_cp = pltpu.make_async_copy(wu_hbm, wu_v, sem_w.at[6])
        wd_cp = pltpu.make_async_copy(wd_hbm, wd_v, sem_w.at[7])

        x_cp.start()
        wq0_cp.start()
        for t0 in range(2):
            k_copy(t0, t0).start()
            for c in range(vchunks):
                v_copy(t0, t0, c).start()
        wq1_cp.start()
        wo_cp.start()
        wr_cp.start()
        wg_cp.start()
        wu_cp.start()
        wd_cp.start()

        o_s[...] = jnp.zeros_like(o_s)
        acc_s[...] = jnp.zeros_like(acc_s)
        x_s[...] = jnp.zeros_like(x_s)
        x_cp.wait()
        x_s[0:B, :] = x_v[...].astype(jnp.float32)
        xn_s[...] = _layernorm(x_s[...]).astype(jnp.bfloat16)
        wq0_cp.wait()

        row_id = lax.broadcasted_iota(jnp.int32, (ROWS, DH), 0)

        def step(t, carry):
            slot = t % 2
            h = t // B
            b = t % B

            @pl.when(t == 2 * B)
            def _():
                wq1_cp.wait()

            @pl.when(t % (2 * B) == 0)
            def _():
                off = pl.multiple_of((t // (2 * B)) * PAIR, 128)
                qq = jnp.dot(xn_s[...], wq_v[:, pl.ds(off, PAIR)],
                             preferred_element_type=jnp.float32)
                q_s[0] = qq[:, :DH].astype(jnp.bfloat16)
                q_s[1] = qq[:, DH:].astype(jnp.bfloat16)

            k_copy(t, slot).wait()
            s = jnp.dot(q_s[h % 2], kbuf[slot], preferred_element_type=jnp.float32)

            @pl.when(t + 2 < NSTEP)
            def _():
                k_copy(t + 2, slot).start()

            s = s * SCALE
            m = jnp.max(s, axis=-1, keepdims=True)
            p = jnp.exp(s - m)
            l = jnp.sum(p, axis=-1, keepdims=True)
            pb = p.astype(jnp.bfloat16)
            inv_l = 1.0 / l
            for c in range(vchunks):
                v_copy(t, slot, c).wait()
                oc = lax.dot_general(
                    pb, vbuf[slot, pl.ds(c * vrows, vrows), :],
                    (((1,), (1,)), ((), ())), preferred_element_type=jnp.float32)
                sel = lax.broadcasted_iota(jnp.int32, (ROWS, vrows), 0) == b
                o_s[:, c * vrows:(c + 1) * vrows] = jnp.where(
                    sel, oc * inv_l, o_s[:, c * vrows:(c + 1) * vrows])

                @pl.when(t + 2 < NSTEP)
                def _():
                    v_copy(t + 2, slot, c).start()

            @pl.when(t == B - 1)
            def _():
                wo_cp.wait()

            @pl.when(b == B - 1)
            def _():
                off = pl.multiple_of(h * DH, 16)
                acc_s[...] += jnp.dot(o_s[...].astype(jnp.bfloat16),
                                      wo_v[pl.ds(off, DH), :],
                                      preferred_element_type=jnp.float32)
            return carry

        lax.fori_loop(0, NSTEP, step, 0)

        wr_cp.wait()
        wg_cp.wait()
        wu_cp.wait()
        wd_cp.wait()
        hres = x_s[...] + acc_s[...]
        hn = _layernorm(hres)
        hb = hn.astype(jnp.bfloat16)
        r = jnp.sum(hn * wr_v[...].astype(jnp.float32), axis=-1, keepdims=True)
        g = jnp.dot(hb, wg_v[...], preferred_element_type=jnp.float32)
        u = jnp.dot(hb, wu_v[...], preferred_element_type=jnp.float32)
        a = (g * jax.nn.sigmoid(g) * u).astype(jnp.bfloat16)
        y = jnp.dot(a, wd_v[...], preferred_element_type=jnp.float32)
        res = hres + hn + y * jax.nn.sigmoid(r)
        out_ref[...] = res[0:B, :].astype(out_ref.dtype)

    return kernel


def _build(vchunks=1):
    kernel = _make_kernel(vchunks)
    bf = jnp.bfloat16
    any_spec = pl.BlockSpec(memory_space=pl.ANY)

    def fn(A_x, A_k_cache, A_v_cache, A_wq, A_wo, B_x, B_w_r, B_w_gate, B_w_up, B_w_down):
        del B_x
        x2 = A_x.reshape(B, D)
        kt = jnp.swapaxes(A_k_cache, 2, 3)
        vt = jnp.swapaxes(A_v_cache, 2, 3)
        wr2 = B_w_r.reshape(1, D)
        out = pl.pallas_call(
            kernel,
            out_shape=jax.ShapeDtypeStruct((B, D), bf),
            in_specs=[any_spec] * 9,
            out_specs=pl.BlockSpec(memory_space=pltpu.VMEM),
            scratch_shapes=[
                pltpu.VMEM((B, D), bf),
                pltpu.VMEM((1, D), bf),
                pltpu.VMEM((D, H * DH), bf),
                pltpu.VMEM((H * DH, D), bf),
                pltpu.VMEM((D, F), bf),
                pltpu.VMEM((D, F), bf),
                pltpu.VMEM((F, D), bf),
                pltpu.VMEM((2, DH, SK), bf),
                pltpu.VMEM((2, DH, SK), bf),
                pltpu.VMEM((ROWS, D), jnp.float32),
                pltpu.VMEM((ROWS, D), bf),
                pltpu.VMEM((2, ROWS, DH), bf),
                pltpu.VMEM((ROWS, DH), jnp.float32),
                pltpu.VMEM((ROWS, D), jnp.float32),
                pltpu.SemaphoreType.DMA((8,)),
                pltpu.SemaphoreType.DMA((2,)),
                pltpu.SemaphoreType.DMA((2, vchunks)),
            ],
            compiler_params=pltpu.CompilerParams(vmem_limit_bytes=100 * 1024 * 1024),
        )(x2, kt, vt, A_wq, A_wo, wr2, B_w_gate, B_w_up, B_w_down)
        return out.reshape(B, 1, D)

    return fn


_impl = _build()


@jax.jit
def pallas_sequential_preLN__mha_block_cached__moe_arch_mod__decode_kernel(
    A_x: jax.Array,
    A_k_cache: jax.Array,
    A_v_cache: jax.Array,
    A_wq: jax.Array,
    A_wo: jax.Array,
    B_x: jax.Array,
    B_w_r: jax.Array,
    B_w_gate: jax.Array,
    B_w_up: jax.Array,
    B_w_down: jax.Array,
):
    return _impl(A_x, A_k_cache, A_v_cache, A_wq, A_wo, B_x, B_w_r, B_w_gate, B_w_up, B_w_down)
```

```python
import jax
import jax.numpy as jnp
from jax import lax
import jax.experimental.pallas as pl
import jax.experimental.pallas.tpu as pltpu

B, H, SK, DH, D, F = 4, 32, 8192, 192, 640, 1536
NSTEP = B * H
CH = 8
NJ = DH // CH
NCHUNK = NSTEP * NJ
LANES = 128
NT = SK // LANES
ROWS = 8
EPS = 1e-5
SCALE = DH ** -0.5
PAIR = 2 * DH
NSUB = 4
SUBC = SK // NSUB
f32 = jnp.float32
bf16 = jnp.bfloat16


WD_GROUPS = ((0, 384), (384, 256), (640, 128))
WD_ROWS = 16


def _layernorm(x):
    m = jnp.mean(x, axis=-1, keepdims=True)
    c = x - m
    v = jnp.mean(c * c, axis=-1, keepdims=True)
    return c / jnp.sqrt(v + EPS)


def _make_kernel(RK, RV, dbg=()):
    A = RK - 1
    assert RV >= A + NJ + 1 and A <= NJ
    WO_PER_IT = 6
    WO_G = 3
    n_wo_pairs = H * NJ // WO_G // 2
    assert n_wo_pairs <= WO_PER_IT * NJ
    FF_PER_IT = 4
    n_gu = D // CH
    n_wd = F // 2 // WD_ROWS
    tail_first = NCHUNK - A

    def kernel(x_hbm, k_hbm, v_hbm, wq_hbm, wo_hbm, wr_hbm, wg_hbm, wu_hbm, wd_hbm,
               out_ref,
               x_v, wr_v, wq_v, wo_v, wg_v, wu_v, wd_v, ring,
               x_s, xn_s, qh_s, qcol_s, s_acc, p_rep, attn_s, h_s,
               sem_misc, sem_wd, sem_ring):

        def base(t):
            return ((t % B) * H + t // B) * NJ

        def pair_start(g, i):
            ks = i % RK
            vs = RK + i % RV
            for c in range(NSUB):
                cols = pl.ds(c * SUBC, SUBC)
                pltpu.make_async_copy(k_hbm.at[g, :, cols], ring.at[ks, :, cols],
                                      sem_ring.at[ks]).start(priority=0)
                pltpu.make_async_copy(v_hbm.at[g, :, cols], ring.at[vs, :, cols],
                                      sem_ring.at[vs]).start(priority=1)

        def chunk_wait(slot):
            pltpu.make_async_copy(ring.at[slot], ring.at[slot], sem_ring.at[slot]).wait()

        def wo_pair_start(n):
            for half in range(2):
                rows = pl.ds(half * (H * NJ // 2) + n * WO_G, WO_G)
                pltpu.make_async_copy(wo_hbm.at[rows], wo_v.at[rows],
                                      sem_misc.at[2]).start(priority=half)

        def gu_pair_start(n):
            rows = pl.ds(pl.multiple_of(n * CH, CH), CH)
            pltpu.make_async_copy(wg_hbm.at[rows], wg_v.at[rows], sem_misc.at[3]).start(priority=0)
            pltpu.make_async_copy(wu_hbm.at[rows], wu_v.at[rows], sem_misc.at[4]).start(priority=1)

        def wd_pair_start(n, grp):
            for half in range(2):
                rows = pl.ds(pl.multiple_of(half * (F // 2) + n * WD_ROWS, WD_ROWS), WD_ROWS)
                pltpu.make_async_copy(wd_hbm.at[rows], wd_v.at[rows],
                                      sem_wd.at[2 * grp + half]).start(priority=half)

        x_cp = pltpu.make_async_copy(x_hbm, x_v, sem_misc.at[0])
        wr_cp = pltpu.make_async_copy(wr_hbm, wr_v, sem_misc.at[1])

        x_cp.start(priority=0)
        wr_cp.start(priority=1)

        def wq_issue(r, carry):
            for c in range(H * DH // SUBC):
                cols = pl.ds(c * SUBC, SUBC)
                for half in range(2):
                    rows = pl.ds(pl.multiple_of(half * (D // 2) + r * CH, CH), CH)
                    pltpu.make_async_copy(wq_hbm.at[rows, cols], wq_v.at[rows, cols],
                                          sem_misc.at[5]).start(priority=half)
            return carry

        lax.fori_loop(0, D // 2 // CH, wq_issue, 0)
        for i in range(A):
            pair_start(i, i)

        s_acc[...] = jnp.zeros_like(s_acc)
        attn_s[...] = jnp.zeros_like(attn_s)
        x_s[...] = jnp.zeros_like(x_s)
        x_cp.wait()
        x_s[0:B, :] = x_v[...].astype(f32)
        xn_s[...] = _layernorm(x_s[...]).astype(bf16)
        pltpu.make_async_copy(wq_hbm, wq_v, sem_misc.at[5]).wait()

        def proj_q(pair):
            off = pl.multiple_of(pair * PAIR, LANES)
            qq = jnp.dot(xn_s[...], wq_v[:, pl.ds(off, PAIR)], preferred_element_type=f32) * SCALE
            qh_s[0] = qq[:, :DH]
            qh_s[1] = qq[:, DH:]

        def prep_q(t):
            row = qh_s[(t // B) % 2, pl.ds(t % B, 1), :]
            qcol_s[...] = jnp.transpose(jnp.broadcast_to(row, (LANES, DH)))

        proj_q(0)
        prep_q(0)

        def k_work(j, slot):
            qc = qcol_s[pl.ds(pl.multiple_of(j * CH, CH), CH), :]
            for c in range(NT):
                sl = slice(c * LANES, (c + 1) * LANES)
                s_acc[:, sl] += ring[slot, :, sl].astype(f32) * qc

        def v_work(j, slot, b, h):
            accs = [None] * 4
            for c in range(NT):
                sl = slice(c * LANES, (c + 1) * LANES)
                tt = ring[slot, :, sl].astype(f32) * p_rep[:, sl]
                accs[c % 4] = tt if accs[c % 4] is None else accs[c % 4] + tt
            acc = (accs[0] + accs[1]) + (accs[2] + accs[3])
            oc = jnp.sum(acc, axis=1, keepdims=True)
            attn_s[b] += oc * wo_v[h * NJ + j].astype(f32)

        def softmax():
            s = jnp.sum(s_acc[...], axis=0, keepdims=True)
            s_acc[...] = jnp.zeros_like(s_acc)
            m = jnp.max(s, axis=-1, keepdims=True)
            p = jnp.exp(s - m)
            l = jnp.sum(p, axis=-1, keepdims=True)
            p_rep[...] = jnp.broadcast_to(p * (1.0 / l), (ROWS, SK))

        def tail_issue(n):
            for u in range(FF_PER_IT):
                m = n * FF_PER_IT + u

                @pl.when(m < n_gu)
                def _():
                    gu_pair_start(m)

                for grp, (r0, nr) in enumerate(WD_GROUPS):
                    lo = n_gu + r0 // WD_ROWS

                    @pl.when(jnp.logical_and(m >= lo, m < lo + nr // WD_ROWS))
                    def _():
                        wd_pair_start(m - n_gu, grp)

        def phase(t, has_k, has_v, first=False, last_k=False):
            i0 = t * NJ
            if has_k:
                kb0 = base(t)
                kb1 = base(jnp.minimum(t + 1, NSTEP - 1))
            if has_v:
                bv = (t - 1) % B
                hv = (t - 1) // B

            def body(j, carry):
                i = i0 + j
                if has_v:
                    vslot = RK + (i - NJ) % RV
                    chunk_wait(vslot)
                if has_k:
                    kslot = i % RK
                    chunk_wait(kslot)
                if has_v and 'nov' not in dbg:
                    v_work(j, vslot, bv, hv)
                if has_k and 'nok' not in dbg:
                    k_work(j, kslot)
                if has_k:
                    jn = j + A
                    g = jnp.where(jn < NJ, kb0 + jn, kb1 + jn - NJ)
                    if last_k:
                        @pl.when(jn < NJ)
                        def _():
                            pair_start(g, i + A)
                    else:
                        pair_start(g, i + A)
                if first:
                    for u in range(WO_PER_IT):
                        n = j * WO_PER_IT + u

                        @pl.when(n < n_wo_pairs)
                        def _():
                            wo_pair_start(n)
                if last_k or not has_k:
                    @pl.when(i >= tail_first)
                    def _():
                        tail_issue(i - tail_first)
                return carry

            lax.fori_loop(0, NJ, body, 0)
            if has_k and 'nosm' not in dbg:
                softmax()
                if not last_k:
                    @pl.when((t + 1) % (2 * B) == 0)
                    def _():
                        proj_q((t + 1) // (2 * B))
                    prep_q(t + 1)

        phase(0, True, False, first=True)
        pltpu.make_async_copy(wo_hbm, wo_v, sem_misc.at[2]).wait()

        def main(t, carry):
            phase(t, True, True)
            return carry

        lax.fori_loop(1, NSTEP - 1, main, 0)
        phase(NSTEP - 1, True, True, last_k=True)
        phase(NSTEP, False, True)

        h_s[...] = x_s[...]
        for b in range(B):
            h_s[b:b + 1, :] += jnp.sum(attn_s[b], axis=0, keepdims=True)
        hres = h_s[...]
        hn = _layernorm(hres)
        hb = hn.astype(bf16)
        wr_cp.wait()
        r = jnp.sum(hn * wr_v[...].astype(f32), axis=-1, keepdims=True)
        pltpu.make_async_copy(wg_hbm, wg_v, sem_misc.at[3]).wait()
        g = jnp.dot(hb, wg_v[...], preferred_element_type=f32)
        pltpu.make_async_copy(wu_hbm, wu_v, sem_misc.at[4]).wait()
        u = jnp.dot(hb, wu_v[...], preferred_element_type=f32)
        a = (g * jax.nn.sigmoid(g) * u).astype(bf16)
        y = None
        for grp, (r0, nr) in enumerate(WD_GROUPS):
            for half in range(2):
                o = half * (F // 2) + r0
                dst = wd_v.at[pl.ds(o, nr)]
                pltpu.make_async_copy(dst, dst, sem_wd.at[2 * grp + half]).wait()
                part = jnp.dot(a[:, o:o + nr], wd_v[pl.ds(o, nr), :], preferred_element_type=f32)
                y = part if y is None else y + part
        res = hres + hn + y * jax.nn.sigmoid(r)
        out_ref[...] = res[0:B, :].astype(out_ref.dtype)

    assert (NSTEP + 1) * NJ - tail_first >= (n_gu + n_wd + FF_PER_IT - 1) // FF_PER_IT
    return kernel


def _build(RK=16, RV=64, dbg=(), checks=False):
    kernel = _make_kernel(RK, RV, dbg)
    any_spec = pl.BlockSpec(memory_space=pl.ANY)

    def fn(A_x, A_k_cache, A_v_cache, A_wq, A_wo, B_x, B_w_r, B_w_gate, B_w_up, B_w_down):
        del B_x
        x2 = A_x.reshape(B, D)
        kt = jnp.swapaxes(A_k_cache, 2, 3).reshape(NCHUNK, CH, SK)
        vt = jnp.swapaxes(A_v_cache, 2, 3).reshape(NCHUNK, CH, SK)
        wo3 = A_wo.reshape(H * NJ, CH, D)
        wr2 = B_w_r.reshape(1, D)
        out = pl.pallas_call(
            kernel,
            out_shape=jax.ShapeDtypeStruct((B, D), bf16),
            in_specs=[any_spec] * 9,
            out_specs=pl.BlockSpec(memory_space=pltpu.VMEM),
            scratch_shapes=[
                pltpu.VMEM((B, D), bf16),
                pltpu.VMEM((1, D), bf16),
                pltpu.VMEM((D, H * DH), bf16),
                pltpu.VMEM((H * NJ, CH, D), bf16),
                pltpu.VMEM((D, F), bf16),
                pltpu.VMEM((D, F), bf16),
                pltpu.VMEM((F, D), bf16),
                pltpu.VMEM((RK + RV, CH, SK), bf16),
                pltpu.VMEM((ROWS, D), f32),
                pltpu.VMEM((ROWS, D), bf16),
                pltpu.VMEM((2, ROWS, DH), f32),
                pltpu.VMEM((DH, LANES), f32),
                pltpu.VMEM((ROWS, SK), f32),
                pltpu.VMEM((ROWS, SK), f32),
                pltpu.VMEM((B, CH, D), f32),
                pltpu.VMEM((ROWS, D), f32),
                pltpu.SemaphoreType.DMA((6,)),
                pltpu.SemaphoreType.DMA((2 * len(WD_GROUPS),)),
                pltpu.SemaphoreType.DMA((RK + RV,)),
            ],
            compiler_params=pltpu.CompilerParams(
                vmem_limit_bytes=100 * 1024 * 1024,
                disable_bounds_checks=not checks,
                disable_semaphore_checks=not checks),
        )(x2, kt, vt, A_wq, wo3, wr2, B_w_gate, B_w_up, B_w_down)
        return out.reshape(B, 1, D)

    return fn


_impl = _build()


@jax.jit
def pallas_sequential_preLN__mha_block_cached__moe_arch_mod__decode_kernel(
    A_x: jax.Array,
    A_k_cache: jax.Array,
    A_v_cache: jax.Array,
    A_wq: jax.Array,
    A_wo: jax.Array,
    B_x: jax.Array,
    B_w_r: jax.Array,
    B_w_gate: jax.Array,
    B_w_up: jax.Array,
    B_w_down: jax.Array,
):
    return _impl(A_x, A_k_cache, A_v_cache, A_wq, A_wo, B_x, B_w_r, B_w_gate, B_w_up, B_w_down)
```

```python
import jax
import jax.numpy as jnp
from jax import lax
import jax.experimental.pallas as pl
import jax.experimental.pallas.tpu as pltpu

B, H, SK, DH, D, F = 4, 32, 8192, 192, 640, 1536
NSTEP = B * H
CH = 8
NJ = DH // CH
NCHUNK = NSTEP * NJ
LANES = 128
NT = SK // LANES
ROWS = 8
EPS = 1e-5
SCALE = DH ** -0.5
PAIR = 2 * DH
NSUB = 4
SUBC = SK // NSUB
f32 = jnp.float32
bf16 = jnp.bfloat16


WD_GROUPS = ((0, 384), (384, 256), (640, 128))
WD_ROWS = 32
GU_ROWS = 16
WO_G = 3
WO_HP = NJ // WO_G


class _NoScope:
    def __enter__(self):
        return self

    def __exit__(self, *a):
        return False


def _layernorm(x):
    m = jnp.mean(x, axis=-1, keepdims=True)
    c = x - m
    v = jnp.mean(c * c, axis=-1, keepdims=True)
    return c / jnp.sqrt(v + EPS)


def _make_kernel(RK, RV, ff, DV, KS, VS, order, dbg=()):
    A = RK - 1
    assert sum(KS) == NT and sum(VS) == NT
    k_off = [sum(KS[:c]) for c in range(len(KS))]
    v_off = [sum(VS[:c]) for c in range(len(VS))]
    cnt = {'k': 0, 'v': 0}
    seq = []
    for w in order:
        lw = w.lower()
        seq.append((lw, cnt[lw], ('kv'.index(lw) + (w != lw)) % 2))
        cnt[lw] += 1
    assert cnt['k'] == len(KS) and cnt['v'] == len(VS)
    assert RV >= A + NJ + 1 and A <= NJ and 0 <= DV <= A
    n_gu = D // GU_ROWS
    n_wd = F // 2 // WD_ROWS
    n_ff = n_gu + n_wd
    tail_first = NCHUNK - A
    ff_k, ff_v = ff
    n_ff_k = (NCHUNK - tail_first) * ff_k

    def kernel(x_hbm, k_hbm, v_hbm, wq_hbm, wo_hbm, wr_hbm, wg_hbm, wu_hbm, wd_hbm,
               out_ref,
               x_v, wr_v, wq_v, wo_v, wg_v, wu_v, wd_v, ring,
               x_s, xn_s, qh_s, qcol_s, s_acc, p_rep, attn_s, h_s,
               sem_misc, sem_wo, sem_wd, sem_ring):

        def scope(name):
            return jax.named_scope(name) if 'scopes' in dbg else _NoScope()

        def base(t):
            if 'seq' in dbg:
                return t * NJ
            return ((t % B) * H + t // B) * NJ

        def pair_start(gk, ik, gv, iv):
            both = ik is not None and iv is not None
            n = 0
            for which, c, prio in seq:
                if which == 'k' and ik is not None:
                    cols = pl.ds(k_off[c] * LANES, KS[c] * LANES)
                    ks = ik % RK
                    pltpu.make_async_copy(k_hbm.at[gk, :, cols], ring.at[ks, :, cols],
                                          sem_ring.at[ks]).start(priority=prio if both else n % 2)
                    n += 1
                if which == 'v' and iv is not None:
                    cols = pl.ds(v_off[c] * LANES, VS[c] * LANES)
                    vs = RK + iv % RV
                    pltpu.make_async_copy(v_hbm.at[gv, :, cols], ring.at[vs, :, cols],
                                          sem_ring.at[vs]).start(priority=prio if both else n % 2)
                    n += 1

        def chunk_wait(slot):
            pltpu.make_async_copy(ring.at[slot], ring.at[slot], sem_ring.at[slot]).wait()

        def wo_pair_start(n):
            for half in range(2):
                rows = pl.ds(half * (H * NJ // 2) + n * WO_G, WO_G)
                pltpu.make_async_copy(wo_hbm.at[rows], wo_v.at[rows],
                                      sem_wo.at[(n // WO_HP) % 2, half]).start(priority=half)

        def wo_wait(hp):
            for half in range(2):
                dst = wo_v.at[pl.ds(half * (H * NJ // 2) + hp * NJ, NJ)]
                pltpu.make_async_copy(dst, dst, sem_wo.at[hp % 2, half]).wait()

        def gu_pair_start(n):
            rows = pl.ds(pl.multiple_of(n * GU_ROWS, GU_ROWS), GU_ROWS)
            pltpu.make_async_copy(wg_hbm.at[rows], wg_v.at[rows], sem_misc.at[3]).start(priority=0)
            pltpu.make_async_copy(wu_hbm.at[rows], wu_v.at[rows], sem_misc.at[4]).start(priority=1)

        def wd_pair_start(n, grp):
            for half in range(2):
                rows = pl.ds(pl.multiple_of(half * (F // 2) + n * WD_ROWS, WD_ROWS), WD_ROWS)
                pltpu.make_async_copy(wd_hbm.at[rows], wd_v.at[rows],
                                      sem_wd.at[2 * grp + half]).start(priority=half)

        x_cp = pltpu.make_async_copy(x_hbm, x_v, sem_misc.at[0])
        wr_cp = pltpu.make_async_copy(wr_hbm, wr_v, sem_misc.at[1])

        x_cp.start(priority=0)
        wr_cp.start(priority=1)

        def wq_issue(r, carry):
            for c in range(H * DH // SUBC):
                cols = pl.ds(c * SUBC, SUBC)
                for half in range(2):
                    rows = pl.ds(pl.multiple_of(half * (D // 2) + r * CH, CH), CH)
                    pltpu.make_async_copy(wq_hbm.at[rows, cols], wq_v.at[rows, cols],
                                          sem_misc.at[5]).start(priority=half)
            return carry

        with scope("wq_issue"):
            lax.fori_loop(0, D // 2 // CH, wq_issue, 0)
        with scope("ringfill"):
            for i in range(A):
                if i >= DV:
                    pair_start(i, i, i - DV, i - DV)
                else:
                    pair_start(i, i, None, None)
            for n in range(WO_HP):
                wo_pair_start(n)

        s_acc[...] = jnp.zeros_like(s_acc)
        attn_s[...] = jnp.zeros_like(attn_s)
        x_s[...] = jnp.zeros_like(x_s)
        x_cp.wait()
        x_s[0:B, :] = x_v[...].astype(f32)
        xn_s[...] = _layernorm(x_s[...]).astype(bf16)
        with scope("wq_wait"):
            pltpu.make_async_copy(wq_hbm, wq_v, sem_misc.at[5]).wait()

        def proj_q(pair):
            off = pl.multiple_of(pair * PAIR, LANES)
            qq = jnp.dot(xn_s[...], wq_v[:, pl.ds(off, PAIR)], preferred_element_type=f32) * SCALE
            qh_s[0] = qq[:, :DH]
            qh_s[1] = qq[:, DH:]

        def prep_q(t):
            row = qh_s[(t // B) % 2, pl.ds(t % B, 1), :]
            qcol_s[...] = jnp.transpose(jnp.broadcast_to(row, (LANES, DH)))

        with scope("q0"):
            proj_q(0)
            prep_q(0)

        def k_work(j, slot):
            qc = qcol_s[pl.ds(pl.multiple_of(j * CH, CH), CH), :]
            for c in range(NT):
                sl = slice(c * LANES, (c + 1) * LANES)
                s_acc[:, sl] += ring[slot, :, sl].astype(f32) * qc

        def v_work(j, slot, b, h):
            accs = [None] * 4
            for c in range(NT):
                sl = slice(c * LANES, (c + 1) * LANES)
                tt = ring[slot, :, sl].astype(f32) * p_rep[:, sl]
                accs[c % 4] = tt if accs[c % 4] is None else accs[c % 4] + tt
            acc = (accs[0] + accs[1]) + (accs[2] + accs[3])
            oc = jnp.sum(acc, axis=1, keepdims=True)
            attn_s[b] += oc * wo_v[h * NJ + j].astype(f32)

        def softmax():
            s = jnp.sum(s_acc[...], axis=0, keepdims=True)
            s_acc[...] = jnp.zeros_like(s_acc)
            m = jnp.max(s, axis=-1, keepdims=True)
            p = jnp.exp(s - m)
            l = jnp.sum(p, axis=-1, keepdims=True)
            p_rep[...] = jnp.broadcast_to(p * (1.0 / l), (ROWS, SK))

        def ff_issue(m):
            @pl.when(m < n_gu)
            def _():
                gu_pair_start(m)

            for grp, (r0, nr) in enumerate(WD_GROUPS):
                lo = n_gu + r0 // WD_ROWS

                @pl.when(jnp.logical_and(m >= lo, m < lo + nr // WD_ROWS))
                def _():
                    wd_pair_start(m - n_gu, grp)

        def phase(t, has_k, has_v, last_k=False):
            i0 = t * NJ
            if has_k:
                kb0 = base(t)
                kb1 = base(jnp.minimum(t + 1, NSTEP - 1))
            if has_v:
                bv = (t - 1) % B
                hv = (t - 1) // B

                if not (last_k or not has_k):
                    @pl.when(jnp.logical_and(bv == 0, hv < (H // 2 if 'nowo' not in dbg else 1)))
                    def _():
                        wo_wait(hv)

                    @pl.when(t <= ((H // 2 - 1) * B if 'nowo' not in dbg else -1))
                    def _():
                        per = WO_HP // B
                        for u in range(per):
                            wo_pair_start(WO_HP + (t - 1) * per + u)

            def body(j, carry):
                i = i0 + j
                if has_v:
                    vslot = RK + (i - NJ) % RV
                    chunk_wait(vslot)
                if has_k:
                    kslot = i % RK
                    chunk_wait(kslot)
                if has_v and 'nov' not in dbg:
                    v_work(j, vslot, bv, hv)
                if has_k and 'nok' not in dbg:
                    k_work(j, kslot)
                if has_k:
                    jn = j + A
                    gk = jnp.where(jn < NJ, kb0 + jn, kb1 + jn - NJ)
                    jv = jn - DV
                    gv = jnp.where(jv < NJ, kb0 + jv, kb1 + jv - NJ)
                    if last_k:
                        @pl.when(jn < NJ)
                        def _():
                            pair_start(gk, i + A, gv, i + A - DV)

                        if DV:
                            @pl.when(jnp.logical_and(jn >= NJ, jv < NJ))
                            def _():
                                pair_start(None, None, gv, i + A - DV)
                    else:
                        pair_start(gk, i + A, gv, i + A - DV)
                if last_k:
                    @pl.when(i >= tail_first)
                    def _():
                        for u in range(ff_k):
                            ff_issue((i - tail_first) * ff_k + u)
                if not has_k:
                    for u in range(ff_v):
                        ff_issue(n_ff_k + j * ff_v + u)
                return carry

            lax.fori_loop(0, NJ, body, 0)
            if has_k and 'nosm' not in dbg:
                softmax()
                if not last_k:
                    @pl.when((t + 1) % (2 * B) == 0)
                    def _():
                        proj_q((t + 1) // (2 * B))
                    prep_q(t + 1)

        with scope("phase0"):
            phase(0, True, False)

        def main(t, carry):
            phase(t, True, True)
            return carry

        with scope("main"):
            lax.fori_loop(1, NSTEP - 1, main, 0)
        with scope("phase127"):
            phase(NSTEP - 1, True, True, last_k=True)
        with scope("phase128"):
            phase(NSTEP, False, True)

        with scope("ln2"):
            h_s[...] = x_s[...]
            for b in range(B):
                h_s[b:b + 1, :] += jnp.sum(attn_s[b], axis=0, keepdims=True)
            hres = h_s[...]
            hn = _layernorm(hres)
            hb = hn.astype(bf16)
            wr_cp.wait()
            wr = wr_v[...].astype(f32)
            rp = hn[:, 0:LANES] * wr[0:1, :]
            for c in range(1, D // LANES):
                rp = rp + hn[:, c * LANES:(c + 1) * LANES] * wr[c:c + 1, :]
            r = jnp.sum(rp, axis=-1, keepdims=True)
        with scope("ff_rest"):
            for m in range(min(n_ff_k + NJ * ff_v, n_ff), n_ff):
                if m < n_gu:
                    gu_pair_start(m)
                else:
                    grp = [k for k, (r0, nr) in enumerate(WD_GROUPS)
                           if r0 <= (m - n_gu) * WD_ROWS < r0 + nr][0]
                    wd_pair_start(m - n_gu, grp)
        with scope("wg_wait"):
            pltpu.make_async_copy(wg_hbm, wg_v, sem_misc.at[3]).wait()
            pltpu.make_async_copy(wu_hbm, wu_v, sem_misc.at[4]).wait()
        with scope("gateup"):
            g = jnp.dot(hb, wg_v[...], preferred_element_type=f32)
            u = jnp.dot(hb, wu_v[...], preferred_element_type=f32)
            a = (g * jax.nn.sigmoid(g) * u).astype(bf16)
        y = None
        for grp, (r0, nr) in enumerate(WD_GROUPS):
            with scope("wd_wait%d" % grp):
                for half in range(2):
                    o = half * (F // 2) + r0
                    dst = wd_v.at[pl.ds(o, nr)]
                    pltpu.make_async_copy(dst, dst, sem_wd.at[2 * grp + half]).wait()
            with scope("wd_mm%d" % grp):
                for half in range(2):
                    o = half * (F // 2) + r0
                    part = jnp.dot(a[:, o:o + nr], wd_v[pl.ds(o, nr), :], preferred_element_type=f32)
                    y = part if y is None else y + part
        with scope("final"):
            res = hres + hn + y * jax.nn.sigmoid(r)
            out_ref[...] = res[0:B, :].astype(out_ref.dtype)

    return kernel


def _build(RK=16, RV=64, ff=(3, 1), DV=0, KS=(16, 31, 17), VS=(14, 30, 20), order='kvkvvk', dbg=(), checks=False):
    kernel = _make_kernel(RK, RV, ff, DV, tuple(KS), tuple(VS), order, dbg)
    any_spec = pl.BlockSpec(memory_space=pl.ANY)

    def fn(A_x, A_k_cache, A_v_cache, A_wq, A_wo, B_x, B_w_r, B_w_gate, B_w_up, B_w_down):
        del B_x
        x2 = A_x.reshape(B, D)
        kt = jnp.swapaxes(A_k_cache, 2, 3).reshape(NCHUNK, CH, SK)
        vt = jnp.swapaxes(A_v_cache, 2, 3).reshape(NCHUNK, CH, SK)
        wo3 = A_wo.reshape(H * NJ, CH, D)
        wr2 = B_w_r.reshape(D // LANES, LANES)
        out = pl.pallas_call(
            kernel,
            out_shape=jax.ShapeDtypeStruct((B, D), bf16),
            in_specs=[any_spec] * 9,
            out_specs=pl.BlockSpec(memory_space=pltpu.VMEM),
            scratch_shapes=[
                pltpu.VMEM((B, D), bf16),
                pltpu.VMEM((D // LANES, LANES), bf16),
                pltpu.VMEM((D, H * DH), bf16),
                pltpu.VMEM((H * NJ, CH, D), bf16),
                pltpu.VMEM((D, F), bf16),
                pltpu.VMEM((D, F), bf16),
                pltpu.VMEM((F, D), bf16),
                pltpu.VMEM((RK + RV, CH, SK), bf16),
                pltpu.VMEM((ROWS, D), f32),
                pltpu.VMEM((ROWS, D), bf16),
                pltpu.VMEM((2, ROWS, DH), f32),
                pltpu.VMEM((DH, LANES), f32),
                pltpu.VMEM((ROWS, SK), f32),
                pltpu.VMEM((ROWS, SK), f32),
                pltpu.VMEM((B, CH, D), f32),
                pltpu.VMEM((ROWS, D), f32),
                pltpu.SemaphoreType.DMA((6,)),
                pltpu.SemaphoreType.DMA((2, 2)),
                pltpu.SemaphoreType.DMA((2 * len(WD_GROUPS),)),
                pltpu.SemaphoreType.DMA((RK + RV,)),
            ],
            compiler_params=pltpu.CompilerParams(
                vmem_limit_bytes=100 * 1024 * 1024,
                disable_bounds_checks=not checks,
                disable_semaphore_checks=not checks),
        )(x2, kt, vt, A_wq, wo3, wr2, B_w_gate, B_w_up, B_w_down)
        return out.reshape(B, 1, D)

    return fn


_impl = _build()


@jax.jit
def pallas_sequential_preLN__mha_block_cached__moe_arch_mod__decode_kernel(
    A_x: jax.Array,
    A_k_cache: jax.Array,
    A_v_cache: jax.Array,
    A_wq: jax.Array,
    A_wo: jax.Array,
    B_x: jax.Array,
    B_w_r: jax.Array,
    B_w_gate: jax.Array,
    B_w_up: jax.Array,
    B_w_down: jax.Array,
):
    return _impl(A_x, A_k_cache, A_v_cache, A_wq, A_wo, B_x, B_w_r, B_w_gate, B_w_up, B_w_down)
```

```python
import jax
import jax.numpy as jnp
from jax import lax
import jax.experimental.pallas as pl
import jax.experimental.pallas.tpu as pltpu

B, H, SK, DH, D, F = 4, 32, 8192, 192, 640, 1536
NSTEP = B * H
CH = 8
NJ = DH // CH
NCHUNK = NSTEP * NJ
LANES = 128
NT = SK // LANES
ROWS = 8
EPS = 1e-5
SCALE = DH ** -0.5
PAIR = 2 * DH
f32 = jnp.float32
bf16 = jnp.bfloat16


WD_ROWS = 32
GU_ROWS = 16
WO_RT = D // LANES
WO_TILES = H * NJ * WO_RT


class _NoScope:
    def __enter__(self):
        return self

    def __exit__(self, *a):
        return False


def _layernorm(x):
    m = jnp.mean(x, axis=-1, keepdims=True)
    c = x - m
    v = jnp.mean(c * c, axis=-1, keepdims=True)
    return c / jnp.sqrt(v + EPS)


def _make_kernel(RK, RV, ff, DV, KS, VS, order, WD_GROUPS, dbg=()):
    A = RK - 1
    assert sum(KS) == NT and sum(VS) == NT
    k_off = [sum(KS[:c]) for c in range(len(KS))]
    v_off = [sum(VS[:c]) for c in range(len(VS))]
    cnt = {'k': 0, 'v': 0}
    seq = []
    for w in order:
        lw = w.lower()
        seq.append((lw, cnt[lw], ('kv'.index(lw) + (w != lw)) % 2))
        cnt[lw] += 1
    assert cnt['k'] == len(KS) and cnt['v'] == len(VS)
    assert RV >= A + NJ + 1 and A <= NJ and 0 <= DV <= A
    period = [(0, k_off[c], KS[c], prio) if w == 'k' else (1, v_off[c], VS[c], prio)
              for w, c, prio in seq]
    WQ_RT = H * DH // LANES
    WQ_SP = 4
    assert WQ_SP * WQ_RT == 3 * NT
    wq_tokens = []
    for per in range(3):
        for st, off, n, prio in period:
            a, e = per * NT + off, per * NT + off + n
            while a < e:
                m = min(e, (a // WQ_RT + 1) * WQ_RT)
                wq_tokens.append((st, a // WQ_RT, a % WQ_RT, m - a, prio))
                a = m
    n_gu = D // GU_ROWS
    n_wd = F // 2 // WD_ROWS
    n_ff = n_gu + n_wd
    tail_first = NCHUNK - A
    ff_k, ff_v = ff
    n_ff_k = (NCHUNK - tail_first) * ff_k

    def kernel(x_hbm, k_hbm, v_hbm, wq_hbm, wo_hbm, wr_hbm, wg_hbm, wu_hbm, wd_hbm,
               out_ref,
               x_v, wr_v, wq_v, wo_v, wg_v, wu_v, wd_v, ring,
               x_s, xn_s, qh_s, qcol_s, s_acc, p_rep, attn_s, h_s,
               sem_misc, sem_wd, sem_ring):

        def scope(name):
            return jax.named_scope(name) if 'scopes' in dbg else _NoScope()

        def base(t):
            if 'seq' in dbg:
                return t * NJ
            return ((t % B) * H + t // B) * NJ

        def pair_start(gk, ik, gv, iv):
            both = ik is not None and iv is not None
            n = 0
            for which, c, prio in seq:
                if which == 'k' and ik is not None:
                    cols = pl.ds(k_off[c] * LANES, KS[c] * LANES)
                    ks = ik % RK
                    pltpu.make_async_copy(k_hbm.at[gk, :, cols], ring.at[ks, :, cols],
                                          sem_ring.at[ks]).start(priority=prio if both else n % 2)
                    n += 1
                if which == 'v' and iv is not None:
                    cols = pl.ds(v_off[c] * LANES, VS[c] * LANES)
                    vs = RK + iv % RV
                    pltpu.make_async_copy(v_hbm.at[gv, :, cols], ring.at[vs, :, cols],
                                          sem_ring.at[vs]).start(priority=prio if both else n % 2)
                    n += 1

        def chunk_wait(slot):
            pltpu.make_async_copy(ring.at[slot], ring.at[slot], sem_ring.at[slot]).wait()

        def wo_issue(per, carry):
            for st, off, n, prio in period:
                rng = pl.ds(st * (WO_TILES // 2) + per * NT + off, n)
                pltpu.make_async_copy(wo_hbm.at[rng], wo_v.at[rng],
                                      sem_misc.at[2]).start(priority=prio)
            return carry

        def gu_pair_start(n):
            rows = pl.ds(pl.multiple_of(n * GU_ROWS, GU_ROWS), GU_ROWS)
            pltpu.make_async_copy(wg_hbm.at[rows], wg_v.at[rows], sem_misc.at[3]).start(priority=0)
            pltpu.make_async_copy(wu_hbm.at[rows], wu_v.at[rows], sem_misc.at[4]).start(priority=1)

        def wd_pair_start(n, grp):
            for half in range(2):
                rows = pl.ds(pl.multiple_of(half * (F // 2) + n * WD_ROWS, WD_ROWS), WD_ROWS)
                pltpu.make_async_copy(wd_hbm.at[rows], wd_v.at[rows],
                                      sem_wd.at[2 * grp + half]).start(priority=half)

        x_cp = pltpu.make_async_copy(x_hbm, x_v, sem_misc.at[0])
        wr_cp = pltpu.make_async_copy(wr_hbm, wr_v, sem_misc.at[1])

        x_cp.start(priority=0)
        wr_cp.start(priority=1)

        def wq_issue(sp, carry):
            for st, rg, c0, n, prio in wq_tokens:
                rows = pl.ds(pl.multiple_of((st * (D // 2 // CH) + sp * WQ_SP + rg) * CH, CH), CH)
                cols = pl.ds(c0 * LANES, n * LANES)
                pltpu.make_async_copy(wq_hbm.at[rows, cols], wq_v.at[rows, cols],
                                      sem_misc.at[5]).start(priority=prio)
            return carry

        with scope("wq_issue"):
            lax.fori_loop(0, D // 2 // CH // WQ_SP, wq_issue, 0)
        with scope("wo_issue"):
            lax.fori_loop(0, WO_TILES // 2 // NT, wo_issue, 0)
        with scope("ringfill"):
            for i in range(A):
                if i >= DV:
                    pair_start(i, i, i - DV, i - DV)
                else:
                    pair_start(i, i, None, None)

        s_acc[...] = jnp.zeros_like(s_acc)
        attn_s[...] = jnp.zeros_like(attn_s)
        x_s[...] = jnp.zeros_like(x_s)
        x_cp.wait()
        x_s[0:B, :] = x_v[...].astype(f32)
        xn_s[...] = _layernorm(x_s[...]).astype(bf16)
        with scope("wq_wait"):
            pltpu.make_async_copy(wq_hbm, wq_v, sem_misc.at[5]).wait()

        def proj_q(pair):
            off = pl.multiple_of(pair * PAIR, LANES)
            qq = jnp.dot(xn_s[...], wq_v[:, pl.ds(off, PAIR)], preferred_element_type=f32) * SCALE
            qh_s[0] = qq[:, :DH]
            qh_s[1] = qq[:, DH:]

        def prep_q(t):
            row = qh_s[(t // B) % 2, pl.ds(t % B, 1), :]
            qcol_s[...] = jnp.transpose(jnp.broadcast_to(row, (LANES, DH)))

        with scope("q0"):
            proj_q(0)
            prep_q(0)

        def k_work(j, slot):
            qc = qcol_s[pl.ds(pl.multiple_of(j * CH, CH), CH), :]
            for c in range(NT):
                sl = slice(c * LANES, (c + 1) * LANES)
                s_acc[:, sl] += ring[slot, :, sl].astype(f32) * qc

        def v_work(j, slot, b, h):
            accs = [None] * 4
            for c in range(NT):
                sl = slice(c * LANES, (c + 1) * LANES)
                tt = ring[slot, :, sl].astype(f32) * p_rep[:, sl]
                accs[c % 4] = tt if accs[c % 4] is None else accs[c % 4] + tt
            acc = (accs[0] + accs[1]) + (accs[2] + accs[3])
            oc = jnp.sum(acc, axis=1, keepdims=True)
            w0 = (h * NJ + j) * WO_RT
            for c in range(WO_RT):
                attn_s[b, :, c * LANES:(c + 1) * LANES] += oc * wo_v[w0 + c].astype(f32)

        def softmax():
            s = jnp.sum(s_acc[...], axis=0, keepdims=True)
            s_acc[...] = jnp.zeros_like(s_acc)
            m = jnp.max(s, axis=-1, keepdims=True)
            p = jnp.exp(s - m)
            l = jnp.sum(p, axis=-1, keepdims=True)
            p_rep[...] = jnp.broadcast_to(p * (1.0 / l), (ROWS, SK))

        def ff_issue(m):
            @pl.when(m < n_gu)
            def _():
                gu_pair_start(m)

            for grp, (r0, nr) in enumerate(WD_GROUPS):
                lo = n_gu + r0 // WD_ROWS

                @pl.when(jnp.logical_and(m >= lo, m < lo + nr // WD_ROWS))
                def _():
                    wd_pair_start(m - n_gu, grp)

        def phase(t, has_k, has_v, last_k=False):
            i0 = t * NJ
            if has_k:
                kb0 = base(t)
                kb1 = base(jnp.minimum(t + 1, NSTEP - 1))
            if has_v:
                bv = (t - 1) % B
                hv = (t - 1) // B


            def body(j, carry):
                i = i0 + j
                if has_v:
                    vslot = RK + (i - NJ) % RV
                    chunk_wait(vslot)
                if has_k:
                    kslot = i % RK
                    chunk_wait(kslot)
                if has_v and 'nov' not in dbg:
                    v_work(j, vslot, bv, hv)
                if has_k and 'nok' not in dbg:
                    k_work(j, kslot)
                if has_k:
                    jn = j + A
                    gk = jnp.where(jn < NJ, kb0 + jn, kb1 + jn - NJ)
                    jv = jn - DV
                    gv = jnp.where(jv < NJ, kb0 + jv, kb1 + jv - NJ)
                    if last_k:
                        @pl.when(jn < NJ)
                        def _():
                            pair_start(gk, i + A, gv, i + A - DV)

                        if DV:
                            @pl.when(jnp.logical_and(jn >= NJ, jv < NJ))
                            def _():
                                pair_start(None, None, gv, i + A - DV)
                    else:
                        pair_start(gk, i + A, gv, i + A - DV)
                if last_k:
                    @pl.when(i >= tail_first)
                    def _():
                        for u in range(ff_k):
                            ff_issue((i - tail_first) * ff_k + u)
                if not has_k:
                    for u in range(ff_v):
                        ff_issue(n_ff_k + j * ff_v + u)
                return carry

            lax.fori_loop(0, NJ, body, 0)
            if has_k and 'nosm' not in dbg:
                softmax()
                if not last_k:
                    @pl.when((t + 1) % (2 * B) == 0)
                    def _():
                        proj_q((t + 1) // (2 * B))
                    prep_q(t + 1)

        with scope("phase0"):
            phase(0, True, False)
        pltpu.make_async_copy(wo_hbm, wo_v, sem_misc.at[2]).wait()

        def main(t, carry):
            phase(t, True, True)
            return carry

        with scope("main"):
            lax.fori_loop(1, NSTEP - 1, main, 0)
        with scope("phase127"):
            phase(NSTEP - 1, True, True, last_k=True)
        with scope("phase128"):
            phase(NSTEP, False, True)

        with scope("ln2"):
            h_s[...] = x_s[...]
            for b in range(B):
                h_s[b:b + 1, :] += jnp.sum(attn_s[b], axis=0, keepdims=True)
            hres = h_s[...]
            hn = _layernorm(hres)
            hb = hn.astype(bf16)
            wr_cp.wait()
            wr = wr_v[...].astype(f32)
            rp = hn[:, 0:LANES] * wr[0:1, :]
            for c in range(1, D // LANES):
                rp = rp + hn[:, c * LANES:(c + 1) * LANES] * wr[c:c + 1, :]
            r = jnp.sum(rp, axis=-1, keepdims=True)
        with scope("ff_rest"):
            for m in range(min(n_ff_k + NJ * ff_v, n_ff), n_ff):
                if m < n_gu:
                    gu_pair_start(m)
                else:
                    grp = [k for k, (r0, nr) in enumerate(WD_GROUPS)
                           if r0 <= (m - n_gu) * WD_ROWS < r0 + nr][0]
                    wd_pair_start(m - n_gu, grp)
        with scope("wg_wait"):
            pltpu.make_async_copy(wg_hbm, wg_v, sem_misc.at[3]).wait()
        with scope("gate"):
            g = jnp.dot(hb, wg_v[...], preferred_element_type=f32)
            g = g * jax.nn.sigmoid(g)
        with scope("wu_wait"):
            pltpu.make_async_copy(wu_hbm, wu_v, sem_misc.at[4]).wait()
        with scope("up"):
            u = jnp.dot(hb, wu_v[...], preferred_element_type=f32)
            a = (g * u).astype(bf16)
        y = None
        for grp, (r0, nr) in enumerate(WD_GROUPS):
            with scope("wd_wait%d" % grp):
                for half in range(2):
                    o = half * (F // 2) + r0
                    dst = wd_v.at[pl.ds(o, nr)]
                    pltpu.make_async_copy(dst, dst, sem_wd.at[2 * grp + half]).wait()
            with scope("wd_mm%d" % grp):
                for half in range(2):
                    o = half * (F // 2) + r0
                    part = jnp.dot(a[:, o:o + nr], wd_v[pl.ds(o, nr), :], preferred_element_type=f32)
                    y = part if y is None else y + part
        with scope("final"):
            res = hres + hn + y * jax.nn.sigmoid(r)
            out_ref[...] = res[0:B, :].astype(out_ref.dtype)

    return kernel


def _build(RK=16, RV=64, ff=(3, 1), DV=0, KS=(16, 31, 17), VS=(14, 30, 20), order='kvkvvk',
           wdg=((0, 384), (384, 256), (640, 128)), dbg=(), checks=False):
    kernel = _make_kernel(RK, RV, ff, DV, tuple(KS), tuple(VS), order, wdg, dbg)
    any_spec = pl.BlockSpec(memory_space=pl.ANY)

    def fn(A_x, A_k_cache, A_v_cache, A_wq, A_wo, B_x, B_w_r, B_w_gate, B_w_up, B_w_down):
        del B_x
        x2 = A_x.reshape(B, D)
        kt = jnp.swapaxes(A_k_cache, 2, 3).reshape(NCHUNK, CH, SK)
        vt = jnp.swapaxes(A_v_cache, 2, 3).reshape(NCHUNK, CH, SK)
        wo3 = A_wo.reshape(H * NJ, CH, WO_RT, LANES).transpose(0, 2, 1, 3).reshape(WO_TILES, CH, LANES)
        wr2 = B_w_r.reshape(D // LANES, LANES)
        out = pl.pallas_call(
            kernel,
            out_shape=jax.ShapeDtypeStruct((B, D), bf16),
            in_specs=[any_spec] * 9,
            out_specs=pl.BlockSpec(memory_space=pltpu.VMEM),
            scratch_shapes=[
                pltpu.VMEM((B, D), bf16),
                pltpu.VMEM((D // LANES, LANES), bf16),
                pltpu.VMEM((D, H * DH), bf16),
                pltpu.VMEM((WO_TILES, CH, LANES), bf16),
                pltpu.VMEM((D, F), bf16),
                pltpu.VMEM((D, F), bf16),
                pltpu.VMEM((F, D), bf16),
                pltpu.VMEM((RK + RV, CH, SK), bf16),
                pltpu.VMEM((ROWS, D), f32),
                pltpu.VMEM((ROWS, D), bf16),
                pltpu.VMEM((2, ROWS, DH), f32),
                pltpu.VMEM((DH, LANES), f32),
                pltpu.VMEM((ROWS, SK), f32),
                pltpu.VMEM((ROWS, SK), f32),
                pltpu.VMEM((B, CH, D), f32),
                pltpu.VMEM((ROWS, D), f32),
                pltpu.SemaphoreType.DMA((6,)),
                pltpu.SemaphoreType.DMA((2 * len(wdg),)),
                pltpu.SemaphoreType.DMA((RK + RV,)),
            ],
            compiler_params=pltpu.CompilerParams(
                vmem_limit_bytes=100 * 1024 * 1024,
                disable_bounds_checks=not checks,
                disable_semaphore_checks=not checks),
        )(x2, kt, vt, A_wq, wo3, wr2, B_w_gate, B_w_up, B_w_down)
        return out.reshape(B, 1, D)

    return fn


_impl = _build()


@jax.jit
def pallas_sequential_preLN__mha_block_cached__moe_arch_mod__decode_kernel(
    A_x: jax.Array,
    A_k_cache: jax.Array,
    A_v_cache: jax.Array,
    A_wq: jax.Array,
    A_wo: jax.Array,
    B_x: jax.Array,
    B_w_r: jax.Array,
    B_w_gate: jax.Array,
    B_w_up: jax.Array,
    B_w_down: jax.Array,
):
    return _impl(A_x, A_k_cache, A_v_cache, A_wq, A_wo, B_x, B_w_r, B_w_gate, B_w_up, B_w_down)
```

```python
import jax
import jax.numpy as jnp
from jax import lax
import jax.experimental.pallas as pl
import jax.experimental.pallas.tpu as pltpu

B, H, SK, DH, D, F = 4, 32, 8192, 192, 640, 1536
LANES = 128
CH = 8
ROWS = 8
NSTEP = B * H
NJ = DH // CH
NCHUNK = NSTEP * NJ
NT = SK // LANES
PAIR = 2 * DH
EPS = 1e-5
SCALE = DH ** -0.5
f32 = jnp.float32
bf16 = jnp.bfloat16

PERIOD = 64
PIECES = ((0, 0, 16), (1, 0, 14), (0, 16, 31), (1, 14, 30), (1, 44, 20), (0, 47, 17))
KV_PIECES = PIECES
RK = 16
RV = 64
AHEAD = RK - 1
GU_ROWS = 16
WD_ROWS = 32
WD_GROUPS = ((0, 384), (384, 256), (640, 128))
FF_K, FF_V = 3, 1

WO_RT = D // LANES
WO_TILES = H * NJ * WO_RT
WQ_RT = H * DH // LANES
WQ_SP = 3 * PERIOD // WQ_RT
N_GU = D // GU_ROWS
N_WD = F // 2 // WD_ROWS
N_FF = N_GU + N_WD
TAIL_FIRST = NCHUNK - AHEAD
N_FF_K = AHEAD * FF_K

assert AHEAD <= NJ and RV >= AHEAD + NJ + 1
assert sum(n for s, _, n in KV_PIECES if s == 0) == NT == sum(n for s, _, n in KV_PIECES if s == 1)
assert WQ_SP * WQ_RT == 3 * PERIOD and (D // 2 // CH) % WQ_SP == 0
assert (WO_TILES // 2) % PERIOD == 0


def _wq_pieces():
    out = []
    for per in range(3):
        for st, off, n in PIECES:
            a, e = per * PERIOD + off, per * PERIOD + off + n
            while a < e:
                m = min(e, (a // WQ_RT + 1) * WQ_RT)
                out.append((st, a // WQ_RT, a % WQ_RT, m - a))
                a = m
    return out


def _layernorm(x):
    m = jnp.mean(x, axis=-1, keepdims=True)
    c = x - m
    v = jnp.mean(c * c, axis=-1, keepdims=True)
    return c / jnp.sqrt(v + EPS)


def _kernel(x_hbm, k_hbm, v_hbm, wq_hbm, wo_hbm, wr_hbm, wg_hbm, wu_hbm, wd_hbm,
            out_ref,
            x_v, wr_v, wq_v, wo_v, wg_v, wu_v, wd_v, ring,
            x_s, xn_s, qh_s, qcol_s, s_acc, p_rep, attn_s, h_s,
            sem_misc, sem_wd, sem_ring):
    SEM_X, SEM_WR, SEM_WO, SEM_WG, SEM_WU, SEM_WQ = range(6)

    def wait_filled(ref, sem):
        pltpu.make_async_copy(ref, ref, sem).wait()

    def base(t):
        return ((t % B) * H + t // B) * NJ

    def kv_start(g, i):
        for st, off, n in KV_PIECES:
            cols = pl.ds(off * LANES, n * LANES)
            src = (k_hbm, v_hbm)[st]
            slot = i % RK if st == 0 else RK + i % RV
            pltpu.make_async_copy(src.at[g, :, cols], ring.at[slot, :, cols],
                                  sem_ring.at[slot]).start(priority=st)

    def wq_issue(sp, carry):
        for st, rg, c0, n in _wq_pieces():
            rows = pl.ds(pl.multiple_of((st * (D // 2 // CH) + sp * WQ_SP + rg) * CH, CH), CH)
            cols = pl.ds(c0 * LANES, n * LANES)
            pltpu.make_async_copy(wq_hbm.at[rows, cols], wq_v.at[rows, cols],
                                  sem_misc.at[SEM_WQ]).start(priority=st)
        return carry

    def wo_issue(per, carry):
        for st, off, n in PIECES:
            rng = pl.ds(st * (WO_TILES // 2) + per * PERIOD + off, n)
            pltpu.make_async_copy(wo_hbm.at[rng], wo_v.at[rng],
                                  sem_misc.at[SEM_WO]).start(priority=st)
        return carry

    def gu_start(n):
        rows = pl.ds(pl.multiple_of(n * GU_ROWS, GU_ROWS), GU_ROWS)
        pltpu.make_async_copy(wg_hbm.at[rows], wg_v.at[rows], sem_misc.at[SEM_WG]).start(priority=0)
        pltpu.make_async_copy(wu_hbm.at[rows], wu_v.at[rows], sem_misc.at[SEM_WU]).start(priority=1)

    def wd_start(n, grp):
        for half in range(2):
            rows = pl.ds(pl.multiple_of(half * (F // 2) + n * WD_ROWS, WD_ROWS), WD_ROWS)
            pltpu.make_async_copy(wd_hbm.at[rows], wd_v.at[rows],
                                  sem_wd.at[2 * grp + half]).start(priority=half)

    def ff_issue(m):
        @pl.when(m < N_GU)
        def _():
            gu_start(m)

        for grp, (r0, nr) in enumerate(WD_GROUPS):
            lo = N_GU + r0 // WD_ROWS

            @pl.when(jnp.logical_and(m >= lo, m < lo + nr // WD_ROWS))
            def _():
                wd_start(m - N_GU, grp)

    x_cp = pltpu.make_async_copy(x_hbm, x_v, sem_misc.at[SEM_X])
    wr_cp = pltpu.make_async_copy(wr_hbm, wr_v, sem_misc.at[SEM_WR])

    lax.fori_loop(0, D // 2 // CH // WQ_SP, wq_issue, 0)
    x_cp.start(priority=0)
    wr_cp.start(priority=1)
    lax.fori_loop(0, WO_TILES // 2 // PERIOD, wo_issue, 0)
    for i in range(AHEAD):
        kv_start(i, i)

    s_acc[...] = jnp.zeros_like(s_acc)
    attn_s[...] = jnp.zeros_like(attn_s)
    x_s[...] = jnp.zeros_like(x_s)
    x_cp.wait()
    x_s[0:B, :] = x_v[...].astype(f32)
    xn_s[...] = _layernorm(x_s[...]).astype(bf16)
    wait_filled(wq_v, sem_misc.at[SEM_WQ])

    def proj_q(pair):
        off = pl.multiple_of(pair * PAIR, LANES)
        qq = jnp.dot(xn_s[...], wq_v[:, pl.ds(off, PAIR)], preferred_element_type=f32) * SCALE
        qh_s[0] = qq[:, :DH]
        qh_s[1] = qq[:, DH:]

    def prep_q(t):
        row = qh_s[(t // B) % 2, pl.ds(t % B, 1), :]
        qcol_s[...] = jnp.transpose(jnp.broadcast_to(row, (LANES, DH)))

    proj_q(0)
    prep_q(0)

    def k_work(j, slot):
        qc = qcol_s[pl.ds(pl.multiple_of(j * CH, CH), CH), :]
        for c in range(NT):
            sl = slice(c * LANES, (c + 1) * LANES)
            s_acc[:, sl] += ring[slot, :, sl].astype(f32) * qc

    def v_work(j, slot, b, h):
        accs = [None] * 4
        for c in range(NT):
            sl = slice(c * LANES, (c + 1) * LANES)
            tt = ring[slot, :, sl].astype(f32) * p_rep[:, sl]
            accs[c % 4] = tt if accs[c % 4] is None else accs[c % 4] + tt
        acc = (accs[0] + accs[1]) + (accs[2] + accs[3])
        oc = jnp.sum(acc, axis=1, keepdims=True)
        w0 = (h * NJ + j) * WO_RT
        for c in range(WO_RT):
            attn_s[b, :, c * LANES:(c + 1) * LANES] += oc * wo_v[w0 + c].astype(f32)

    def softmax():
        s = jnp.sum(s_acc[...], axis=0, keepdims=True)
        s_acc[...] = jnp.zeros_like(s_acc)
        m = jnp.max(s, axis=-1, keepdims=True)
        p = jnp.exp(s - m)
        l = jnp.sum(p, axis=-1, keepdims=True)
        p_rep[...] = jnp.broadcast_to(p * (1.0 / l), (ROWS, SK))

    def phase(t, has_k, has_v, last_k=False):
        i0 = t * NJ
        if has_k:
            g0 = base(t)
            g1 = base(jnp.minimum(t + 1, NSTEP - 1))
        if has_v:
            bv = (t - 1) % B
            hv = (t - 1) // B

        def body(j, carry):
            i = i0 + j
            if has_v:
                vslot = RK + (i - NJ) % RV
                wait_filled(ring.at[vslot], sem_ring.at[vslot])
            if has_k:
                kslot = i % RK
                wait_filled(ring.at[kslot], sem_ring.at[kslot])
            if has_v:
                v_work(j, vslot, bv, hv)
            if has_k:
                k_work(j, kslot)
                jn = j + AHEAD
                g = jnp.where(jn < NJ, g0 + jn, g1 + jn - NJ)
                if last_k:
                    @pl.when(jn < NJ)
                    def _():
                        kv_start(g, i + AHEAD)

                    @pl.when(i >= TAIL_FIRST)
                    def _():
                        for u in range(FF_K):
                            ff_issue((i - TAIL_FIRST) * FF_K + u)
                else:
                    kv_start(g, i + AHEAD)
            else:
                for u in range(FF_V):
                    ff_issue(N_FF_K + j * FF_V + u)
            return carry

        lax.fori_loop(0, NJ, body, 0)
        if has_k:
            softmax()
            if not last_k:
                @pl.when((t + 1) % (2 * B) == 0)
                def _():
                    proj_q((t + 1) // (2 * B))

                prep_q(t + 1)

    phase(0, True, False)
    wait_filled(wo_v, sem_misc.at[SEM_WO])

    def main(t, carry):
        phase(t, True, True)
        return carry

    lax.fori_loop(1, NSTEP - 1, main, 0)
    phase(NSTEP - 1, True, True, last_k=True)
    phase(NSTEP, False, True)

    h_s[...] = x_s[...]
    for b in range(B):
        h_s[b:b + 1, :] += jnp.sum(attn_s[b], axis=0, keepdims=True)
    hres = h_s[...]
    hn = _layernorm(hres)
    hb = hn.astype(bf16)
    wr_cp.wait()
    wr = wr_v[...].astype(f32)
    rp = hn[:, 0:LANES] * wr[0:1, :]
    for c in range(1, D // LANES):
        rp = rp + hn[:, c * LANES:(c + 1) * LANES] * wr[c:c + 1, :]
    r = jnp.sum(rp, axis=-1, keepdims=True)
    for m in range(min(N_FF_K + NJ * FF_V, N_FF), N_FF):
        ff_issue(m)
    wait_filled(wg_v, sem_misc.at[SEM_WG])
    g = jnp.dot(hb, wg_v[...], preferred_element_type=f32)
    g = g * jax.nn.sigmoid(g)
    wait_filled(wu_v, sem_misc.at[SEM_WU])
    u = jnp.dot(hb, wu_v[...], preferred_element_type=f32)
    a = (g * u).astype(bf16)
    y = None
    for grp, (r0, nr) in enumerate(WD_GROUPS):
        for half in range(2):
            wait_filled(wd_v.at[pl.ds(half * (F // 2) + r0, nr)], sem_wd.at[2 * grp + half])
        for half in range(2):
            o = half * (F // 2) + r0
            part = jnp.dot(a[:, o:o + nr], wd_v[pl.ds(o, nr), :], preferred_element_type=f32)
            y = part if y is None else y + part
    res = hres + hn + y * jax.nn.sigmoid(r)
    out_ref[...] = res[0:B, :].astype(out_ref.dtype)


def _call(A_x, A_k_cache, A_v_cache, A_wq, A_wo, B_w_r, B_w_gate, B_w_up, B_w_down, **call_kwargs):
    x2 = A_x.reshape(B, D)
    kt = jnp.swapaxes(A_k_cache, 2, 3).reshape(NCHUNK, CH, SK)
    vt = jnp.swapaxes(A_v_cache, 2, 3).reshape(NCHUNK, CH, SK)
    wo3 = A_wo.reshape(H * NJ, CH, WO_RT, LANES).transpose(0, 2, 1, 3).reshape(WO_TILES, CH, LANES)
    wr2 = B_w_r.reshape(D // LANES, LANES)
    out = pl.pallas_call(
        _kernel,
        out_shape=jax.ShapeDtypeStruct((B, D), bf16),
        in_specs=[pl.BlockSpec(memory_space=pl.ANY)] * 9,
        out_specs=pl.BlockSpec(memory_space=pltpu.VMEM),
        scratch_shapes=[
            pltpu.VMEM((B, D), bf16),
            pltpu.VMEM((D // LANES, LANES), bf16),
            pltpu.VMEM((D, H * DH), bf16),
            pltpu.VMEM((WO_TILES, CH, LANES), bf16),
            pltpu.VMEM((D, F), bf16),
            pltpu.VMEM((D, F), bf16),
            pltpu.VMEM((F, D), bf16),
            pltpu.VMEM((RK + RV, CH, SK), bf16),
            pltpu.VMEM((ROWS, D), f32),
            pltpu.VMEM((ROWS, D), bf16),
            pltpu.VMEM((2, ROWS, DH), f32),
            pltpu.VMEM((DH, LANES), f32),
            pltpu.VMEM((ROWS, SK), f32),
            pltpu.VMEM((ROWS, SK), f32),
            pltpu.VMEM((B, CH, D), f32),
            pltpu.VMEM((ROWS, D), f32),
            pltpu.SemaphoreType.DMA((6,)),
            pltpu.SemaphoreType.DMA((2 * len(WD_GROUPS),)),
            pltpu.SemaphoreType.DMA((RK + RV,)),
        ],
        compiler_params=pltpu.CompilerParams(
            vmem_limit_bytes=64 * 1024 * 1024,
            disable_bounds_checks=True,
            disable_semaphore_checks=True),
        **call_kwargs,
    )(x2, kt, vt, A_wq, wo3, wr2, B_w_gate, B_w_up, B_w_down)
    return out.reshape(B, 1, D)


@jax.jit
def pallas_sequential_preLN__mha_block_cached__moe_arch_mod__decode_kernel(
    A_x: jax.Array,
    A_k_cache: jax.Array,
    A_v_cache: jax.Array,
    A_wq: jax.Array,
    A_wo: jax.Array,
    B_x: jax.Array,
    B_w_r: jax.Array,
    B_w_gate: jax.Array,
    B_w_up: jax.Array,
    B_w_down: jax.Array,
):
    del B_x
    return _call(A_x, A_k_cache, A_v_cache, A_wq, A_wo, B_w_r, B_w_gate, B_w_up, B_w_down)
```

```python
import jax
import jax.numpy as jnp
from jax import lax
import jax.experimental.pallas as pl
import jax.experimental.pallas.tpu as pltpu

B, H, SK, DH, D, F = 4, 32, 8192, 192, 640, 1536
LANES = 128
CH = 8
ROWS = 8
NSTEP = B * H
NJ = DH // CH
NCHUNK = NSTEP * NJ
NT = SK // LANES
PAIR = 2 * DH
EPS = 1e-5
SCALE = DH ** -0.5
f32 = jnp.float32
bf16 = jnp.bfloat16

PERIOD = 64
PIECES = ((0, 0, 16), (1, 0, 14), (0, 16, 31), (1, 14, 30), (1, 44, 20), (0, 47, 17))
KV_PIECES = ((0, 0, 0, 15), (1, 1, 44, 20), (0, 0, 15, 1), (1, 0, 0, 12), (0, 0, 16, 31),
             (1, 0, 12, 20), (0, 0, 47, 1), (1, 0, 32, 12), (0, 0, 48, 16))
RK = 16
RV = 64
AHEAD = RK - 1
GU_ROWS = 16
WD_ROWS = 32
WD_GROUPS = ((0, 384), (384, 256), (640, 128))
FF_K, FF_V = 3, 1

WO_RT = D // LANES
WO_TILES = H * NJ * WO_RT
WQ_RT = H * DH // LANES
WQ_SP = 3 * PERIOD // WQ_RT
N_GU = D // GU_ROWS
N_WD = F // 2 // WD_ROWS
N_FF = N_GU + N_WD
TAIL_FIRST = NCHUNK - AHEAD
N_FF_K = AHEAD * FF_K

assert AHEAD <= NJ and RV >= AHEAD + NJ + 1
assert sum(n for s, _, _, n in KV_PIECES if s == 0) == NT == sum(n for s, _, _, n in KV_PIECES if s == 1)
assert WQ_SP * WQ_RT == 3 * PERIOD and (D // 2 // CH) % WQ_SP == 0
assert (WO_TILES // 2) % PERIOD == 0


def _wq_pieces():
    out = []
    for per in range(3):
        for st, off, n in PIECES:
            a, e = per * PERIOD + off, per * PERIOD + off + n
            while a < e:
                m = min(e, (a // WQ_RT + 1) * WQ_RT)
                out.append((st, a // WQ_RT, a % WQ_RT, m - a))
                a = m
    return out


def _layernorm(x):
    m = jnp.mean(x, axis=-1, keepdims=True)
    c = x - m
    v = jnp.mean(c * c, axis=-1, keepdims=True)
    return c / jnp.sqrt(v + EPS)


def _kernel(x_hbm, k_hbm, v_hbm, wq_hbm, wo_hbm, wr_hbm, wg_hbm, wu_hbm, wd_hbm,
            out_ref,
            x_v, wr_v, wq_v, wo_v, wg_v, wu_v, wd_v, ring,
            x_s, xn_s, qh_s, qcol_s, s_acc, p_rep, attn_s, h_s,
            sem_misc, sem_wd, sem_ring):
    SEM_X, SEM_WR, SEM_WO, SEM_WG, SEM_WU, SEM_WQ = range(6)

    def wait_filled(ref, sem):
        pltpu.make_async_copy(ref, ref, sem).wait()

    def base(t):
        return ((t % B) * H + t // B) * NJ

    def kv_start(g, i, g_prev, lags=(0, 1)):
        for st, lag, off, n in KV_PIECES:
            if lag in lags:
                cols = pl.ds(off * LANES, n * LANES)
                slot = i % RK if st == 0 else RK + (i - lag) % RV
                pltpu.make_async_copy((k_hbm, v_hbm)[st].at[g_prev if lag else g, :, cols],
                                      ring.at[slot, :, cols],
                                      sem_ring.at[slot]).start(priority=st)

    def wq_issue(sp, carry):
        for st, rg, c0, n in _wq_pieces():
            rows = pl.ds(pl.multiple_of((st * (D // 2 // CH) + sp * WQ_SP + rg) * CH, CH), CH)
            cols = pl.ds(c0 * LANES, n * LANES)
            pltpu.make_async_copy(wq_hbm.at[rows, cols], wq_v.at[rows, cols],
                                  sem_misc.at[SEM_WQ]).start(priority=st)
        return carry

    def wo_issue(per, carry):
        for st, off, n in PIECES:
            rng = pl.ds(st * (WO_TILES // 2) + per * PERIOD + off, n)
            pltpu.make_async_copy(wo_hbm.at[rng], wo_v.at[rng],
                                  sem_misc.at[SEM_WO]).start(priority=st)
        return carry

    def gu_start(n):
        rows = pl.ds(pl.multiple_of(n * GU_ROWS, GU_ROWS), GU_ROWS)
        pltpu.make_async_copy(wg_hbm.at[rows], wg_v.at[rows], sem_misc.at[SEM_WG]).start(priority=0)
        pltpu.make_async_copy(wu_hbm.at[rows], wu_v.at[rows], sem_misc.at[SEM_WU]).start(priority=1)

    def wd_start(n, grp):
        for half in range(2):
            rows = pl.ds(pl.multiple_of(half * (F // 2) + n * WD_ROWS, WD_ROWS), WD_ROWS)
            pltpu.make_async_copy(wd_hbm.at[rows], wd_v.at[rows],
                                  sem_wd.at[2 * grp + half]).start(priority=half)

    def ff_issue(m):
        @pl.when(m < N_GU)
        def _():
            gu_start(m)

        for grp, (r0, nr) in enumerate(WD_GROUPS):
            lo = N_GU + r0 // WD_ROWS

            @pl.when(jnp.logical_and(m >= lo, m < lo + nr // WD_ROWS))
            def _():
                wd_start(m - N_GU, grp)

    x_cp = pltpu.make_async_copy(x_hbm, x_v, sem_misc.at[SEM_X])
    wr_cp = pltpu.make_async_copy(wr_hbm, wr_v, sem_misc.at[SEM_WR])

    lax.fori_loop(0, D // 2 // CH // WQ_SP, wq_issue, 0)
    x_cp.start(priority=0)
    wr_cp.start(priority=1)
    lax.fori_loop(0, WO_TILES // 2 // PERIOD, wo_issue, 0)
    for i in range(AHEAD):
        kv_start(i, i, i - 1, lags=(0, 1) if i else (0,))

    s_acc[...] = jnp.zeros_like(s_acc)
    attn_s[...] = jnp.zeros_like(attn_s)
    x_s[...] = jnp.zeros_like(x_s)
    x_cp.wait()
    x_s[0:B, :] = x_v[...].astype(f32)
    xn_s[...] = _layernorm(x_s[...]).astype(bf16)
    wait_filled(wq_v, sem_misc.at[SEM_WQ])

    def proj_q(pair):
        off = pl.multiple_of(pair * PAIR, LANES)
        qq = jnp.dot(xn_s[...], wq_v[:, pl.ds(off, PAIR)], preferred_element_type=f32) * SCALE
        qh_s[0] = qq[:, :DH]
        qh_s[1] = qq[:, DH:]

    def prep_q(t):
        row = qh_s[(t // B) % 2, pl.ds(t % B, 1), :]
        qcol_s[...] = jnp.transpose(jnp.broadcast_to(row, (LANES, DH)))

    proj_q(0)
    prep_q(0)

    def k_work(j, slot):
        qc = qcol_s[pl.ds(pl.multiple_of(j * CH, CH), CH), :]
        for c in range(NT):
            sl = slice(c * LANES, (c + 1) * LANES)
            s_acc[:, sl] += ring[slot, :, sl].astype(f32) * qc

    def v_work(j, slot, b, h):
        accs = [None] * 4
        for c in range(NT):
            sl = slice(c * LANES, (c + 1) * LANES)
            tt = ring[slot, :, sl].astype(f32) * p_rep[:, sl]
            accs[c % 4] = tt if accs[c % 4] is None else accs[c % 4] + tt
        acc = (accs[0] + accs[1]) + (accs[2] + accs[3])
        oc = jnp.sum(acc, axis=1, keepdims=True)
        w0 = (h * NJ + j) * WO_RT
        for c in range(WO_RT):
            attn_s[b, :, c * LANES:(c + 1) * LANES] += oc * wo_v[w0 + c].astype(f32)

    def softmax():
        s = jnp.sum(s_acc[...], axis=0, keepdims=True)
        s_acc[...] = jnp.zeros_like(s_acc)
        m = jnp.max(s, axis=-1, keepdims=True)
        p = jnp.exp(s - m)
        l = jnp.sum(p, axis=-1, keepdims=True)
        p_rep[...] = jnp.broadcast_to(p * (1.0 / l), (ROWS, SK))

    def phase(t, has_k, has_v, last_k=False):
        i0 = t * NJ
        if has_k:
            g0 = base(t)
            g1 = base(jnp.minimum(t + 1, NSTEP - 1))
        if has_v:
            bv = (t - 1) % B
            hv = (t - 1) // B

        def body(j, carry):
            i = i0 + j
            if has_v:
                vslot = RK + (i - NJ) % RV
                wait_filled(ring.at[vslot], sem_ring.at[vslot])
            if has_k:
                kslot = i % RK
                wait_filled(ring.at[kslot], sem_ring.at[kslot])
            if has_v:
                v_work(j, vslot, bv, hv)
            if has_k:
                k_work(j, kslot)
                jn = j + AHEAD
                g = jnp.where(jn < NJ, g0 + jn, g1 + jn - NJ)
                g_prev = jnp.where(jn <= NJ, g0 + jn - 1, g1 + jn - 1 - NJ)
                if last_k:
                    @pl.when(jn < NJ)
                    def _():
                        kv_start(g, i + AHEAD, g_prev)

                    @pl.when(jn == NJ)
                    def _():
                        kv_start(g, i + AHEAD, g_prev, lags=(1,))

                    @pl.when(i >= TAIL_FIRST)
                    def _():
                        for u in range(FF_K):
                            ff_issue((i - TAIL_FIRST) * FF_K + u)
                else:
                    kv_start(g, i + AHEAD, g_prev)
            else:
                for u in range(FF_V):
                    ff_issue(N_FF_K + j * FF_V + u)
            return carry

        lax.fori_loop(0, NJ, body, 0)
        if has_k:
            softmax()
            if not last_k:
                @pl.when((t + 1) % (2 * B) == 0)
                def _():
                    proj_q((t + 1) // (2 * B))

                prep_q(t + 1)

    phase(0, True, False)
    wait_filled(wo_v, sem_misc.at[SEM_WO])

    def main(t, carry):
        phase(t, True, True)
        return carry

    lax.fori_loop(1, NSTEP - 1, main, 0)
    phase(NSTEP - 1, True, True, last_k=True)
    phase(NSTEP, False, True)

    h_s[...] = x_s[...]
    for b in range(B):
        h_s[b:b + 1, :] += jnp.sum(attn_s[b], axis=0, keepdims=True)
    hres = h_s[...]
    hn = _layernorm(hres)
    hb = hn.astype(bf16)
    wr_cp.wait()
    wr = wr_v[...].astype(f32)
    rp = hn[:, 0:LANES] * wr[0:1, :]
    for c in range(1, D // LANES):
        rp = rp + hn[:, c * LANES:(c + 1) * LANES] * wr[c:c + 1, :]
    r = jnp.sum(rp, axis=-1, keepdims=True)
    for m in range(min(N_FF_K + NJ * FF_V, N_FF), N_FF):
        ff_issue(m)
    wait_filled(wg_v, sem_misc.at[SEM_WG])
    g = jnp.dot(hb, wg_v[...], preferred_element_type=f32)
    g = g * jax.nn.sigmoid(g)
    wait_filled(wu_v, sem_misc.at[SEM_WU])
    u = jnp.dot(hb, wu_v[...], preferred_element_type=f32)
    a = (g * u).astype(bf16)
    y = None
    for grp, (r0, nr) in enumerate(WD_GROUPS):
        for half in range(2):
            wait_filled(wd_v.at[pl.ds(half * (F // 2) + r0, nr)], sem_wd.at[2 * grp + half])
        for half in range(2):
            o = half * (F // 2) + r0
            part = jnp.dot(a[:, o:o + nr], wd_v[pl.ds(o, nr), :], preferred_element_type=f32)
            y = part if y is None else y + part
    res = hres + hn + y * jax.nn.sigmoid(r)
    out_ref[...] = res[0:B, :].astype(out_ref.dtype)


def _call(A_x, A_k_cache, A_v_cache, A_wq, A_wo, B_w_r, B_w_gate, B_w_up, B_w_down, **call_kwargs):
    x2 = A_x.reshape(B, D)
    kt = jnp.swapaxes(A_k_cache, 2, 3).reshape(NCHUNK, CH, SK)
    vt = jnp.swapaxes(A_v_cache, 2, 3).reshape(NCHUNK, CH, SK)
    wo3 = A_wo.reshape(H * NJ, CH, WO_RT, LANES).transpose(0, 2, 1, 3).reshape(WO_TILES, CH, LANES)
    wr2 = B_w_r.reshape(D // LANES, LANES)
    out = pl.pallas_call(
        _kernel,
        out_shape=jax.ShapeDtypeStruct((B, D), bf16),
        in_specs=[pl.BlockSpec(memory_space=pl.ANY)] * 9,
        out_specs=pl.BlockSpec(memory_space=pltpu.VMEM),
        scratch_shapes=[
            pltpu.VMEM((B, D), bf16),
            pltpu.VMEM((D // LANES, LANES), bf16),
            pltpu.VMEM((D, H * DH), bf16),
            pltpu.VMEM((WO_TILES, CH, LANES), bf16),
            pltpu.VMEM((D, F), bf16),
            pltpu.VMEM((D, F), bf16),
            pltpu.VMEM((F, D), bf16),
            pltpu.VMEM((RK + RV, CH, SK), bf16),
            pltpu.VMEM((ROWS, D), f32),
            pltpu.VMEM((ROWS, D), bf16),
            pltpu.VMEM((2, ROWS, DH), f32),
            pltpu.VMEM((DH, LANES), f32),
            pltpu.VMEM((ROWS, SK), f32),
            pltpu.VMEM((ROWS, SK), f32),
            pltpu.VMEM((B, CH, D), f32),
            pltpu.VMEM((ROWS, D), f32),
            pltpu.SemaphoreType.DMA((6,)),
            pltpu.SemaphoreType.DMA((2 * len(WD_GROUPS),)),
            pltpu.SemaphoreType.DMA((RK + RV,)),
        ],
        compiler_params=pltpu.CompilerParams(
            vmem_limit_bytes=64 * 1024 * 1024,
            disable_bounds_checks=True,
            disable_semaphore_checks=True),
        **call_kwargs,
    )(x2, kt, vt, A_wq, wo3, wr2, B_w_gate, B_w_up, B_w_down)
    return out.reshape(B, 1, D)


@jax.jit
def pallas_sequential_preLN__mha_block_cached__moe_arch_mod__decode_kernel(
    A_x: jax.Array,
    A_k_cache: jax.Array,
    A_v_cache: jax.Array,
    A_wq: jax.Array,
    A_wo: jax.Array,
    B_x: jax.Array,
    B_w_r: jax.Array,
    B_w_gate: jax.Array,
    B_w_up: jax.Array,
    B_w_down: jax.Array,
):
    del B_x
    return _call(A_x, A_k_cache, A_v_cache, A_wq, A_wo, B_w_r, B_w_gate, B_w_up, B_w_down)
```

```python
import jax
import jax.numpy as jnp
from jax import lax
import jax.experimental.pallas as pl
import jax.experimental.pallas.tpu as pltpu

B, H, SK, DH, D, F = 4, 32, 8192, 192, 640, 1536
LANES = 128
CH = 8
ROWS = 8
NSTEP = B * H
NJ = DH // CH
NCHUNK = NSTEP * NJ
NT = SK // LANES
PAIR = 2 * DH
EPS = 1e-5
SCALE = DH ** -0.5
f32 = jnp.float32
bf16 = jnp.bfloat16

PERIOD = 64
PIECES = ((0, 0, 16), (1, 0, 14), (0, 16, 31), (1, 14, 30), (1, 44, 20), (0, 47, 17))
KV_PIECES = ((0, 0, 0, 15), (1, 1, 44, 20), (0, 0, 15, 1), (1, 0, 0, 12), (0, 0, 16, 31),
             (1, 0, 12, 20), (0, 0, 47, 1), (1, 0, 32, 12), (0, 0, 48, 16))
RK = 16
RV = 64
AHEAD = RK - 1
GU_ROWS = 16
WD_ROWS = 32
WD_GROUPS = ((0, 384), (384, 256), (640, 128))
FF_K, FF_V = 3, 1

WO_RT = D // LANES
WO_TILES = H * NJ * WO_RT
WQ_RT = H * DH // LANES
WQ_SP = 3 * PERIOD // WQ_RT
N_GU = D // GU_ROWS
N_WD = F // 2 // WD_ROWS
N_FF = N_GU + N_WD
TAIL_FIRST = NCHUNK - AHEAD
N_FF_K = AHEAD * FF_K

assert AHEAD <= NJ and RV >= AHEAD + NJ + 1
assert sum(n for s, _, _, n in KV_PIECES if s == 0) == NT == sum(n for s, _, _, n in KV_PIECES if s == 1)
assert WQ_SP * WQ_RT == 3 * PERIOD and (D // 2 // CH) % WQ_SP == 0
assert (WO_TILES // 2) % PERIOD == 0


def _wq_pieces():
    out = []
    for per in range(3):
        for st, off, n in PIECES:
            a, e = per * PERIOD + off, per * PERIOD + off + n
            while a < e:
                m = min(e, (a // WQ_RT + 1) * WQ_RT)
                out.append((st, a // WQ_RT, a % WQ_RT, m - a))
                a = m
    return out


def _layernorm(x):
    m = jnp.mean(x, axis=-1, keepdims=True)
    c = x - m
    v = jnp.mean(c * c, axis=-1, keepdims=True)
    return c / jnp.sqrt(v + EPS)


def _kernel(x_hbm, k_hbm, v_hbm, wq_hbm, wo_hbm, wr_hbm, wg_hbm, wu_hbm, wd_hbm,
            out_ref,
            x_v, wr_v, wq_v, wo_v, wg_v, wu_v, wd_v, ring,
            x_s, xn_s, qh_s, qcol_s, s_acc, p_rep, attn_s, h_s,
            sem_misc, sem_wd, sem_ring):
    SEM_X, SEM_WR, SEM_WO, SEM_WG, SEM_WU, SEM_WQ = range(6)

    def wait_filled(ref, sem):
        pltpu.make_async_copy(ref, ref, sem).wait()

    def kv_start(i, lags=(0, 1)):
        for st, lag, off, n in KV_PIECES:
            if lag in lags:
                cols = pl.ds(off * LANES, n * LANES)
                slot = i % RK if st == 0 else RK + (i - lag) % RV
                pltpu.make_async_copy((k_hbm, v_hbm)[st].at[i - lag, :, cols],
                                      ring.at[slot, :, cols],
                                      sem_ring.at[slot]).start(priority=st)

    def wq_issue(sp, carry):
        for st, rg, c0, n in _wq_pieces():
            rows = pl.ds(pl.multiple_of((st * (D // 2 // CH) + sp * WQ_SP + rg) * CH, CH), CH)
            cols = pl.ds(c0 * LANES, n * LANES)
            pltpu.make_async_copy(wq_hbm.at[rows, cols], wq_v.at[rows, cols],
                                  sem_misc.at[SEM_WQ]).start(priority=st)
        return carry

    def wo_issue(per, carry):
        for st, off, n in PIECES:
            rng = pl.ds(st * (WO_TILES // 2) + per * PERIOD + off, n)
            pltpu.make_async_copy(wo_hbm.at[rng], wo_v.at[rng],
                                  sem_misc.at[SEM_WO]).start(priority=st)
        return carry

    def gu_start(n):
        rows = pl.ds(pl.multiple_of(n * GU_ROWS, GU_ROWS), GU_ROWS)
        pltpu.make_async_copy(wg_hbm.at[rows], wg_v.at[rows], sem_misc.at[SEM_WG]).start(priority=0)
        pltpu.make_async_copy(wu_hbm.at[rows], wu_v.at[rows], sem_misc.at[SEM_WU]).start(priority=1)

    def wd_start(n, grp):
        for half in range(2):
            rows = pl.ds(pl.multiple_of(half * (F // 2) + n * WD_ROWS, WD_ROWS), WD_ROWS)
            pltpu.make_async_copy(wd_hbm.at[rows], wd_v.at[rows],
                                  sem_wd.at[2 * grp + half]).start(priority=half)

    def ff_issue(m):
        @pl.when(m < N_GU)
        def _():
            gu_start(m)

        for grp, (r0, nr) in enumerate(WD_GROUPS):
            lo = N_GU + r0 // WD_ROWS

            @pl.when(jnp.logical_and(m >= lo, m < lo + nr // WD_ROWS))
            def _():
                wd_start(m - N_GU, grp)

    x_cp = pltpu.make_async_copy(x_hbm, x_v, sem_misc.at[SEM_X])
    wr_cp = pltpu.make_async_copy(wr_hbm, wr_v, sem_misc.at[SEM_WR])

    lax.fori_loop(0, D // 2 // CH // WQ_SP, wq_issue, 0)
    x_cp.start(priority=0)
    wr_cp.start(priority=1)
    lax.fori_loop(0, WO_TILES // 2 // PERIOD, wo_issue, 0)
    for i in range(AHEAD):
        kv_start(i, lags=(0, 1) if i else (0,))

    s_acc[...] = jnp.zeros_like(s_acc)
    attn_s[...] = jnp.zeros_like(attn_s)
    x_s[...] = jnp.zeros_like(x_s)
    x_cp.wait()
    x_s[0:B, :] = x_v[...].astype(f32)
    xn_s[...] = _layernorm(x_s[...]).astype(bf16)
    wait_filled(wq_v, sem_misc.at[SEM_WQ])

    def proj_q(pair):
        off = pl.multiple_of(pair * PAIR, LANES)
        qq = jnp.dot(xn_s[...], wq_v[:, pl.ds(off, PAIR)], preferred_element_type=f32) * SCALE
        qh_s[2 * pair] = qq[:, :DH]
        qh_s[2 * pair + 1] = qq[:, DH:]

    def prep_q(t):
        row = qh_s[t % H, pl.ds(t // H, 1), :]
        qcol_s[...] = jnp.transpose(jnp.broadcast_to(row, (LANES, DH)))

    proj_q(0)
    prep_q(0)

    def k_work(j, slot):
        qc = qcol_s[pl.ds(pl.multiple_of(j * CH, CH), CH), :]
        for c in range(NT):
            sl = slice(c * LANES, (c + 1) * LANES)
            s_acc[:, sl] += ring[slot, :, sl].astype(f32) * qc

    def v_work(j, slot, b, h):
        accs = [None] * 4
        for c in range(NT):
            sl = slice(c * LANES, (c + 1) * LANES)
            tt = ring[slot, :, sl].astype(f32) * p_rep[:, sl]
            accs[c % 4] = tt if accs[c % 4] is None else accs[c % 4] + tt
        acc = (accs[0] + accs[1]) + (accs[2] + accs[3])
        oc = jnp.sum(acc, axis=1, keepdims=True)
        w0 = (h * NJ + j) * WO_RT
        for c in range(WO_RT):
            attn_s[b, :, c * LANES:(c + 1) * LANES] += oc * wo_v[w0 + c].astype(f32)

    def softmax():
        s = jnp.sum(s_acc[...], axis=0, keepdims=True)
        s_acc[...] = jnp.zeros_like(s_acc)
        m = jnp.max(s, axis=-1, keepdims=True)
        p = jnp.exp(s - m)
        l = jnp.sum(p, axis=-1, keepdims=True)
        p_rep[...] = jnp.broadcast_to(p * (1.0 / l), (ROWS, SK))

    def phase(t, has_k, has_v, last_k=False):
        i0 = t * NJ
        if has_v:
            bv = (t - 1) // H
            hv = (t - 1) % H

        def body(j, carry):
            i = i0 + j
            if has_v:
                vslot = RK + (i - NJ) % RV
                wait_filled(ring.at[vslot], sem_ring.at[vslot])
            if has_k:
                kslot = i % RK
                wait_filled(ring.at[kslot], sem_ring.at[kslot])
            if has_v:
                v_work(j, vslot, bv, hv)
            if has_k:
                k_work(j, kslot)
                if last_k:
                    @pl.when(i < TAIL_FIRST)
                    def _():
                        kv_start(i + AHEAD)

                    @pl.when(i == TAIL_FIRST)
                    def _():
                        kv_start(i + AHEAD, lags=(1,))

                    @pl.when(i >= TAIL_FIRST)
                    def _():
                        for u in range(FF_K):
                            ff_issue((i - TAIL_FIRST) * FF_K + u)
                else:
                    kv_start(i + AHEAD)
            else:
                for u in range(FF_V):
                    ff_issue(N_FF_K + j * FF_V + u)
            return carry

        lax.fori_loop(0, NJ, body, 0)
        if has_k:
            softmax()
            if not last_k:
                @pl.when(jnp.logical_and((t + 1) % 2 == 0, t + 1 < H))
                def _():
                    proj_q((t + 1) // 2)

                prep_q(t + 1)

    phase(0, True, False)
    wait_filled(wo_v, sem_misc.at[SEM_WO])

    def main(t, carry):
        phase(t, True, True)
        return carry

    lax.fori_loop(1, NSTEP - 1, main, 0)
    phase(NSTEP - 1, True, True, last_k=True)
    phase(NSTEP, False, True)

    h_s[...] = x_s[...]
    for b in range(B):
        h_s[b:b + 1, :] += jnp.sum(attn_s[b], axis=0, keepdims=True)
    hres = h_s[...]
    hn = _layernorm(hres)
    hb = hn.astype(bf16)
    wr_cp.wait()
    wr = wr_v[...].astype(f32)
    rp = hn[:, 0:LANES] * wr[0:1, :]
    for c in range(1, D // LANES):
        rp = rp + hn[:, c * LANES:(c + 1) * LANES] * wr[c:c + 1, :]
    r = jnp.sum(rp, axis=-1, keepdims=True)
    for m in range(min(N_FF_K + NJ * FF_V, N_FF), N_FF):
        ff_issue(m)
    wait_filled(wg_v, sem_misc.at[SEM_WG])
    g = jnp.dot(hb, wg_v[...], preferred_element_type=f32)
    g = g * jax.nn.sigmoid(g)
    wait_filled(wu_v, sem_misc.at[SEM_WU])
    u = jnp.dot(hb, wu_v[...], preferred_element_type=f32)
    a = (g * u).astype(bf16)
    y = None
    for grp, (r0, nr) in enumerate(WD_GROUPS):
        for half in range(2):
            wait_filled(wd_v.at[pl.ds(half * (F // 2) + r0, nr)], sem_wd.at[2 * grp + half])
        for half in range(2):
            o = half * (F // 2) + r0
            part = jnp.dot(a[:, o:o + nr], wd_v[pl.ds(o, nr), :], preferred_element_type=f32)
            y = part if y is None else y + part
    res = hres + hn + y * jax.nn.sigmoid(r)
    out_ref[...] = res[0:B, :].astype(out_ref.dtype)


def _call(A_x, A_k_cache, A_v_cache, A_wq, A_wo, B_w_r, B_w_gate, B_w_up, B_w_down, **call_kwargs):
    x2 = A_x.reshape(B, D)
    kt = jnp.swapaxes(A_k_cache, 2, 3).reshape(NCHUNK, CH, SK)
    vt = jnp.swapaxes(A_v_cache, 2, 3).reshape(NCHUNK, CH, SK)
    wo3 = A_wo.reshape(H * NJ, CH, WO_RT, LANES).transpose(0, 2, 1, 3).reshape(WO_TILES, CH, LANES)
    wr2 = B_w_r.reshape(D // LANES, LANES)
    out = pl.pallas_call(
        _kernel,
        out_shape=jax.ShapeDtypeStruct((B, D), bf16),
        in_specs=[pl.BlockSpec(memory_space=pl.ANY)] * 9,
        out_specs=pl.BlockSpec(memory_space=pltpu.VMEM),
        scratch_shapes=[
            pltpu.VMEM((B, D), bf16),
            pltpu.VMEM((D // LANES, LANES), bf16),
            pltpu.VMEM((D, H * DH), bf16),
            pltpu.VMEM((WO_TILES, CH, LANES), bf16),
            pltpu.VMEM((D, F), bf16),
            pltpu.VMEM((D, F), bf16),
            pltpu.VMEM((F, D), bf16),
            pltpu.VMEM((RK + RV, CH, SK), bf16),
            pltpu.VMEM((ROWS, D), f32),
            pltpu.VMEM((ROWS, D), bf16),
            pltpu.VMEM((H, ROWS, DH), f32),
            pltpu.VMEM((DH, LANES), f32),
            pltpu.VMEM((ROWS, SK), f32),
            pltpu.VMEM((ROWS, SK), f32),
            pltpu.VMEM((B, CH, D), f32),
            pltpu.VMEM((ROWS, D), f32),
            pltpu.SemaphoreType.DMA((6,)),
            pltpu.SemaphoreType.DMA((2 * len(WD_GROUPS),)),
            pltpu.SemaphoreType.DMA((RK + RV,)),
        ],
        compiler_params=pltpu.CompilerParams(
            vmem_limit_bytes=64 * 1024 * 1024,
            disable_bounds_checks=True,
            disable_semaphore_checks=True),
        **call_kwargs,
    )(x2, kt, vt, A_wq, wo3, wr2, B_w_gate, B_w_up, B_w_down)
    return out.reshape(B, 1, D)


@jax.jit
def pallas_sequential_preLN__mha_block_cached__moe_arch_mod__decode_kernel(
    A_x: jax.Array,
    A_k_cache: jax.Array,
    A_v_cache: jax.Array,
    A_wq: jax.Array,
    A_wo: jax.Array,
    B_x: jax.Array,
    B_w_r: jax.Array,
    B_w_gate: jax.Array,
    B_w_up: jax.Array,
    B_w_down: jax.Array,
):
    del B_x
    return _call(A_x, A_k_cache, A_v_cache, A_wq, A_wo, B_w_r, B_w_gate, B_w_up, B_w_down)
```

```python
import jax
import jax.numpy as jnp
from jax import lax
import jax.experimental.pallas as pl
import jax.experimental.pallas.tpu as pltpu

B, H, SK, DH, D, F = 4, 32, 8192, 192, 640, 1536
LANES = 128
CH = 8
ROWS = 8
NSTEP = B * H
NJ = DH // CH
NCHUNK = NSTEP * NJ
NT = SK // LANES
PAIR = 2 * DH
EPS = 1e-5
SCALE = DH ** -0.5
f32 = jnp.float32
bf16 = jnp.bfloat16

PERIOD = 64
PIECES = ((0, 0, 16), (1, 0, 14), (0, 16, 31), (1, 14, 30), (1, 44, 20), (0, 47, 17))
KV_LEAD = (16, 19)
KV_PIECES = ((0, 0, 31), (1, 0, 29), (0, 31, 1), (1, 29, 3),
             (0, 32, 31), (1, 32, 29), (0, 63, 1), (1, 61, 3))
RK = 16
RV = 64
GU_ROWS = 16
WD_ROWS = 32
WD_GROUPS = ((0, 384), (384, 256), (640, 128))
FF_K, FF_V = 3, 1

WO_RT = D // LANES
WO_TILES = H * NJ * WO_RT
WQ_RT = H * DH // LANES
WQ_SP = 3 * PERIOD // WQ_RT
N_GU = D // GU_ROWS
N_WD = F // 2 // WD_ROWS
N_FF = N_GU + N_WD
LAST_ISSUE = NCHUNK - RK
N_FF_K = (RK - 1) * FF_K

assert RK <= NJ and RV >= RK + NJ + 1
assert sum(n for s, _, n in KV_PIECES if s == 0) == NT == sum(n for s, _, n in KV_PIECES if s == 1)
assert WQ_SP * WQ_RT == 3 * PERIOD and (D // 2 // CH) % WQ_SP == 0
assert (WO_TILES // 2) % PERIOD == 0


def _wq_pieces():
    out = []
    for per in range(3):
        for st, off, n in PIECES:
            a, e = per * PERIOD + off, per * PERIOD + off + n
            while a < e:
                m = min(e, (a // WQ_RT + 1) * WQ_RT)
                out.append((st, a // WQ_RT, a % WQ_RT, m - a))
                a = m
    return out


def _layernorm(x):
    m = jnp.mean(x, axis=-1, keepdims=True)
    c = x - m
    v = jnp.mean(c * c, axis=-1, keepdims=True)
    return c / jnp.sqrt(v + EPS)


def _kernel(x_hbm, k_hbm, v_hbm, wq_hbm, wo_hbm, wr_hbm, wg_hbm, wu_hbm, wd_hbm,
            out_ref,
            x_v, wr_v, wq_v, wo_v, wg_v, wu_v, wd_v, ring,
            x_s, xn_s, qh_s, qcol_s, s_acc, p_rep, attn_s, h_s,
            sem_misc, sem_wd, sem_ring):
    SEM_X, SEM_WR, SEM_WO, SEM_WG, SEM_WU, SEM_WQ = range(6)

    def wait_filled(ref, sem):
        pltpu.make_async_copy(ref, ref, sem).wait()

    def slot_of(st, n):
        return n % RK if st == 0 else RK + n % RV

    def kv_start(n, part=None):
        for st, off, cnt in KV_PIECES:
            lo, hi = off, off + cnt
            if part == 'first':
                lo = max(lo, KV_LEAD[st])
            if part == 'last':
                hi = min(hi, KV_LEAD[st])
            if lo < hi:
                slot = slot_of(st, n)
                pltpu.make_async_copy(
                    (k_hbm, v_hbm)[st].at[pl.ds(n * NT - KV_LEAD[st] + lo, hi - lo)],
                    ring.at[slot, pl.ds(lo, hi - lo)], sem_ring.at[slot]).start(priority=st)

    def kv_wait(st, n, part=None):
        slot = slot_of(st, n)
        lo = KV_LEAD[st] if part == 'first' else 0
        hi = KV_LEAD[st] if part == 'last' else NT
        wait_filled(ring.at[slot, pl.ds(lo, hi - lo)], sem_ring.at[slot])

    def chunk_tile(st, n, c):
        pos = KV_LEAD[st] + c
        if pos < NT:
            return ring[slot_of(st, n), pos]
        return ring[slot_of(st, n + 1), pos - NT]

    def wq_issue(sp, carry):
        for st, rg, c0, n in _wq_pieces():
            rows = pl.ds(pl.multiple_of((st * (D // 2 // CH) + sp * WQ_SP + rg) * CH, CH), CH)
            cols = pl.ds(c0 * LANES, n * LANES)
            pltpu.make_async_copy(wq_hbm.at[rows, cols], wq_v.at[rows, cols],
                                  sem_misc.at[SEM_WQ]).start(priority=st)
        return carry

    def wo_issue(per, carry):
        for st, off, n in PIECES:
            rng = pl.ds(st * (WO_TILES // 2) + per * PERIOD + off, n)
            pltpu.make_async_copy(wo_hbm.at[rng], wo_v.at[rng],
                                  sem_misc.at[SEM_WO]).start(priority=st)
        return carry

    def gu_start(n):
        rows = pl.ds(pl.multiple_of(n * GU_ROWS, GU_ROWS), GU_ROWS)
        pltpu.make_async_copy(wg_hbm.at[rows], wg_v.at[rows], sem_misc.at[SEM_WG]).start(priority=0)
        pltpu.make_async_copy(wu_hbm.at[rows], wu_v.at[rows], sem_misc.at[SEM_WU]).start(priority=1)

    def wd_start(n, grp):
        for half in range(2):
            rows = pl.ds(pl.multiple_of(half * (F // 2) + n * WD_ROWS, WD_ROWS), WD_ROWS)
            pltpu.make_async_copy(wd_hbm.at[rows], wd_v.at[rows],
                                  sem_wd.at[2 * grp + half]).start(priority=half)

    def ff_issue(m):
        @pl.when(m < N_GU)
        def _():
            gu_start(m)

        for grp, (r0, nr) in enumerate(WD_GROUPS):
            lo = N_GU + r0 // WD_ROWS

            @pl.when(jnp.logical_and(m >= lo, m < lo + nr // WD_ROWS))
            def _():
                wd_start(m - N_GU, grp)

    x_cp = pltpu.make_async_copy(x_hbm, x_v, sem_misc.at[SEM_X])
    wr_cp = pltpu.make_async_copy(wr_hbm, wr_v, sem_misc.at[SEM_WR])

    lax.fori_loop(0, D // 2 // CH // WQ_SP, wq_issue, 0)
    x_cp.start(priority=0)
    wr_cp.start(priority=1)
    lax.fori_loop(0, WO_TILES // 2 // PERIOD, wo_issue, 0)
    kv_start(0, 'first')
    for n in range(1, RK):
        kv_start(n)

    s_acc[...] = jnp.zeros_like(s_acc)
    attn_s[...] = jnp.zeros_like(attn_s)
    x_s[...] = jnp.zeros_like(x_s)
    x_cp.wait()
    x_s[0:B, :] = x_v[...].astype(f32)
    xn_s[...] = _layernorm(x_s[...]).astype(bf16)
    wait_filled(wq_v, sem_misc.at[SEM_WQ])

    def proj_q(pair):
        off = pl.multiple_of(pair * PAIR, LANES)
        qq = jnp.dot(xn_s[...], wq_v[:, pl.ds(off, PAIR)], preferred_element_type=f32) * SCALE
        qh_s[2 * pair] = qq[:, :DH]
        qh_s[2 * pair + 1] = qq[:, DH:]

    def prep_q(t):
        row = qh_s[t % H, pl.ds(t // H, 1), :]
        qcol_s[...] = jnp.transpose(jnp.broadcast_to(row, (LANES, DH)))

    proj_q(0)
    prep_q(0)

    def k_work(j, n):
        qc = qcol_s[pl.ds(pl.multiple_of(j * CH, CH), CH), :]
        for c in range(NT):
            sl = slice(c * LANES, (c + 1) * LANES)
            s_acc[:, sl] += chunk_tile(0, n, c).astype(f32) * qc

    def v_work(j, n, b, h):
        accs = [None] * 4
        for c in range(NT):
            sl = slice(c * LANES, (c + 1) * LANES)
            tt = chunk_tile(1, n, c).astype(f32) * p_rep[:, sl]
            accs[c % 4] = tt if accs[c % 4] is None else accs[c % 4] + tt
        acc = (accs[0] + accs[1]) + (accs[2] + accs[3])
        oc = jnp.sum(acc, axis=1, keepdims=True)
        w0 = (h * NJ + j) * WO_RT
        for c in range(WO_RT):
            attn_s[b, :, c * LANES:(c + 1) * LANES] += oc * wo_v[w0 + c].astype(f32)

    def softmax():
        s = jnp.sum(s_acc[...], axis=0, keepdims=True)
        s_acc[...] = jnp.zeros_like(s_acc)
        m = jnp.max(s, axis=-1, keepdims=True)
        p = jnp.exp(s - m)
        l = jnp.sum(p, axis=-1, keepdims=True)
        p_rep[...] = jnp.broadcast_to(p * (1.0 / l), (ROWS, SK))

    def phase(t, has_k, has_v, last_k=False):
        i0 = t * NJ
        if has_v:
            bv = (t - 1) // H
            hv = (t - 1) % H

        def body(j, carry):
            i = i0 + j
            if has_v:
                if has_k:
                    kv_wait(1, i - NJ + 1)
                else:
                    @pl.when(j < NJ - 1)
                    def _():
                        kv_wait(1, i - NJ + 1)

                    @pl.when(j == NJ - 1)
                    def _():
                        kv_wait(1, i - NJ + 1, 'last')
            if has_k:
                if last_k:
                    @pl.when(j < NJ - 1)
                    def _():
                        kv_wait(0, i + 1)

                    @pl.when(j == NJ - 1)
                    def _():
                        kv_wait(0, i + 1, 'last')
                else:
                    kv_wait(0, i + 1)
            if has_v:
                v_work(j, i - NJ, bv, hv)
            if has_k:
                k_work(j, i)
                if last_k:
                    @pl.when(i < LAST_ISSUE)
                    def _():
                        kv_start(i + RK)

                    @pl.when(i == LAST_ISSUE)
                    def _():
                        kv_start(i + RK, 'last')

                    @pl.when(i > LAST_ISSUE)
                    def _():
                        for u in range(FF_K):
                            ff_issue((i - LAST_ISSUE - 1) * FF_K + u)
                else:
                    kv_start(i + RK)
            else:
                for u in range(FF_V):
                    ff_issue(N_FF_K + j * FF_V + u)
            return carry

        lax.fori_loop(0, NJ, body, 0)
        if has_k:
            softmax()
            if not last_k:
                @pl.when(jnp.logical_and((t + 1) % 2 == 0, t + 1 < H))
                def _():
                    proj_q((t + 1) // 2)

                prep_q(t + 1)

    kv_wait(0, 0, 'first')
    phase(0, True, False)
    wait_filled(wo_v, sem_misc.at[SEM_WO])
    kv_wait(1, 0, 'first')

    def main(t, carry):
        phase(t, True, True)
        return carry

    lax.fori_loop(1, NSTEP - 1, main, 0)
    phase(NSTEP - 1, True, True, last_k=True)
    phase(NSTEP, False, True)

    h_s[...] = x_s[...]
    for b in range(B):
        h_s[b:b + 1, :] += jnp.sum(attn_s[b], axis=0, keepdims=True)
    hres = h_s[...]
    hn = _layernorm(hres)
    hb = hn.astype(bf16)
    wr_cp.wait()
    wr = wr_v[...].astype(f32)
    rp = hn[:, 0:LANES] * wr[0:1, :]
    for c in range(1, D // LANES):
        rp = rp + hn[:, c * LANES:(c + 1) * LANES] * wr[c:c + 1, :]
    r = jnp.sum(rp, axis=-1, keepdims=True)
    for m in range(min(N_FF_K + NJ * FF_V, N_FF), N_FF):
        ff_issue(m)
    wait_filled(wg_v, sem_misc.at[SEM_WG])
    g = jnp.dot(hb, wg_v[...], preferred_element_type=f32)
    g = g * jax.nn.sigmoid(g)
    wait_filled(wu_v, sem_misc.at[SEM_WU])
    u = jnp.dot(hb, wu_v[...], preferred_element_type=f32)
    a = (g * u).astype(bf16)
    y = None
    for grp, (r0, nr) in enumerate(WD_GROUPS):
        for half in range(2):
            wait_filled(wd_v.at[pl.ds(half * (F // 2) + r0, nr)], sem_wd.at[2 * grp + half])
        for half in range(2):
            o = half * (F // 2) + r0
            part = jnp.dot(a[:, o:o + nr], wd_v[pl.ds(o, nr), :], preferred_element_type=f32)
            y = part if y is None else y + part
    res = hres + hn + y * jax.nn.sigmoid(r)
    out_ref[...] = res[0:B, :].astype(out_ref.dtype)


def _call(A_x, A_k_cache, A_v_cache, A_wq, A_wo, B_w_r, B_w_gate, B_w_up, B_w_down, **call_kwargs):
    def tiles(cache):
        t = jnp.swapaxes(cache, 2, 3).reshape(NCHUNK, CH, NT, LANES)
        return t.transpose(0, 2, 1, 3).reshape(NCHUNK * NT, CH, LANES)

    x2 = A_x.reshape(B, D)
    kt = tiles(A_k_cache)
    vt = tiles(A_v_cache)
    wo3 = A_wo.reshape(H * NJ, CH, WO_RT, LANES).transpose(0, 2, 1, 3).reshape(WO_TILES, CH, LANES)
    wr2 = B_w_r.reshape(D // LANES, LANES)
    out = pl.pallas_call(
        _kernel,
        out_shape=jax.ShapeDtypeStruct((B, D), bf16),
        in_specs=[pl.BlockSpec(memory_space=pl.ANY)] * 9,
        out_specs=pl.BlockSpec(memory_space=pltpu.VMEM),
        scratch_shapes=[
            pltpu.VMEM((B, D), bf16),
            pltpu.VMEM((D // LANES, LANES), bf16),
            pltpu.VMEM((D, H * DH), bf16),
            pltpu.VMEM((WO_TILES, CH, LANES), bf16),
            pltpu.VMEM((D, F), bf16),
            pltpu.VMEM((D, F), bf16),
            pltpu.VMEM((F, D), bf16),
            pltpu.VMEM((RK + RV, NT, CH, LANES), bf16),
            pltpu.VMEM((ROWS, D), f32),
            pltpu.VMEM((ROWS, D), bf16),
            pltpu.VMEM((H, ROWS, DH), f32),
            pltpu.VMEM((DH, LANES), f32),
            pltpu.VMEM((ROWS, SK), f32),
            pltpu.VMEM((ROWS, SK), f32),
            pltpu.VMEM((B, CH, D), f32),
            pltpu.VMEM((ROWS, D), f32),
            pltpu.SemaphoreType.DMA((6,)),
            pltpu.SemaphoreType.DMA((2 * len(WD_GROUPS),)),
            pltpu.SemaphoreType.DMA((RK + RV,)),
        ],
        compiler_params=pltpu.CompilerParams(
            vmem_limit_bytes=64 * 1024 * 1024,
            disable_bounds_checks=True,
            disable_semaphore_checks=True),
        **call_kwargs,
    )(x2, kt, vt, A_wq, wo3, wr2, B_w_gate, B_w_up, B_w_down)
    return out.reshape(B, 1, D)


@jax.jit
def pallas_sequential_preLN__mha_block_cached__moe_arch_mod__decode_kernel(
    A_x: jax.Array,
    A_k_cache: jax.Array,
    A_v_cache: jax.Array,
    A_wq: jax.Array,
    A_wo: jax.Array,
    B_x: jax.Array,
    B_w_r: jax.Array,
    B_w_gate: jax.Array,
    B_w_up: jax.Array,
    B_w_down: jax.Array,
):
    del B_x
    return _call(A_x, A_k_cache, A_v_cache, A_wq, A_wo, B_w_r, B_w_gate, B_w_up, B_w_down)
```
